```python
import jax
import jax.numpy as jnp

def _softmax(x, axis=-1):
    return jax.nn.softmax(x, axis=axis)
def _gelu(x):
    return jax.nn.gelu(x, approximate=True)
def _silu(x):
    return jax.nn.silu(x)
def _sigmoid(x):
    return jax.nn.sigmoid(x)
def _layernorm(x, axis=-1, eps=1e-5):
    m = jnp.mean(x, axis=axis, keepdims=True)
    v = jnp.var(x, axis=axis, keepdims=True)
    return (x - m) / jnp.sqrt(v + eps)
def _scatter_add(tgt, idx, src, axis=0):
    return tgt.at[idx].add(src)
def _segment_sum(src, seg, n):
    return jax.ops.segment_sum(src, seg, n)
class _Rng:
    def __init__(self, key):
        self._k = key
    def _next(self):
        self._k, sub = jax.random.split(self._k)
        return sub
    def normal(self, shape):
        return jax.random.normal(self._next(), shape, dtype=jnp.bfloat16)
    def randint(self, lo, hi, shape):
        return jax.random.randint(self._next(), shape, lo, hi, dtype=jnp.int32)
    def uniform(self, shape, lo=0.0, hi=1.0):
        return jax.random.uniform(self._next(), shape, jnp.bfloat16, lo, hi)
    def permutation(self, n):
        return jax.random.permutation(self._next(), n)


kernel_name = 'interleave_layers__sliding_local_dilated__softmax_full_mha__prompt'

def setup_inputs():
    _rng = _Rng(jax.random.key(int.from_bytes(__import__("os").urandom(4), "little")))
    _w = (lambda a: (lambda t: t.astype(jnp.bfloat16) if jnp.issubdtype(t.dtype, jnp.floating) else t)(jnp.asarray(a)))
    def _A_setup():
        B, S, D = 1, 2048, 1024
        return {
            "x": _w((lambda *s: _rng.normal(s) * 0.05)(B, S, D)),
            "wqkv": _w((lambda *s: _rng.normal(s) * 0.05)(D, 3 * D)),
            "wo": _w((lambda *s: _rng.normal(s) * 0.05)(D, D)),
        }
    _A_in = _A_setup()

    def _B_setup():
        B, S, D = 1, 2048, 1024
        return {
            "x": _w((lambda *s: _rng.normal(s) * 0.05)(B, S, D)),
            "wqkv": _w((lambda *s: _rng.normal(s) * 0.05)(D, 3 * D)),
            "wo": _w((lambda *s: _rng.normal(s) * 0.05)(D, D)),
        }
    _B_in = _B_setup()

    return {
        "A_x": _A_in["x"],
        "A_wqkv": _A_in["wqkv"],
        "A_wo": _A_in["wo"],
        "B_x": _B_in["x"],
        "B_wqkv": _B_in["wqkv"],
        "B_wo": _B_in["wo"],
    }

def reference(A_x, A_wqkv, A_wo, B_x, B_wqkv, B_wo):
    def _A_ref(x, wqkv, wo):
        B, S, D = x.shape
        H = 32; Dh = D // H
        W, dil = 8, 2
        qkv = (lambda x, *d: x.transpose(*d))((x @ wqkv).reshape(B, S, 3, H, Dh), 2, 0, 3, 1, 4)
        q, k, v = qkv[0], qkv[1], qkv[2]
        scale = Dh ** -0.5
        pos = jnp.arange(S)
        off = jnp.arange(W) * dil
        idx = pos[:, None] - off[None, :]
        mask = idx >= 0
        idx_c = jnp.where(mask, idx, 0).reshape(-1)
        kg = k[:, :, idx_c, :].reshape(B, H, S, W, Dh)
        vg = v[:, :, idx_c, :].reshape(B, H, S, W, Dh)
        logits = jnp.einsum("bhsd,bhswd->bhsw", q, kg) * scale
        logits = jnp.where(mask[None, None, :, :], logits, -1e9)
        attn = _softmax(logits, axis=-1)
        o = jnp.einsum("bhsw,bhswd->bhsd", attn, vg)
        return (lambda x, *d: x.transpose(*d))(o, 0, 2, 1, 3).reshape(B, S, D) @ wo

    def _B_ref(x, wqkv, wo):
        B, S, D = x.shape
        H = 32; Dh = D // H
        qkv = (lambda x, *d: x.transpose(*d))((x @ wqkv).reshape(B, S, 3, H, Dh), 2, 0, 3, 1, 4)
        q, k, v = qkv[0], qkv[1], qkv[2]
        scale = Dh ** -0.5
        scores = jnp.einsum("bhqd,bhkd->bhqk", q, k) * scale
        p = _softmax(scores, axis=-1)
        o = jnp.einsum("bhqk,bhkd->bhqd", p, v)
        return (lambda x, *d: x.transpose(*d))(o, 0, 2, 1, 3).reshape(B, S, D) @ wo

    x = A_x
    x = x + _A_ref(_layernorm(x, axis=-1), A_wqkv, A_wo)
    x = x + _B_ref(_layernorm(x, axis=-1), B_wqkv, B_wo)
    x = x + _A_ref(_layernorm(x, axis=-1), A_wqkv, A_wo)
    x = x + _B_ref(_layernorm(x, axis=-1), B_wqkv, B_wo)
    return x
```

```python
import math

import jax
import jax.numpy as jnp
from jax import lax
import jax.experimental.pallas as pl
import jax.experimental.pallas.tpu as pltpu

S = 2048
D = 1024
H = 32
DH = D // H
WIN, DIL = 8, 2
EPS = 1e-5
NG = D // 128
BT = 512
NT = S // BT
CK = 128
LOG2E = math.log2(math.e)
QSCALE = DH ** -0.5 * LOG2E
MASKED = -1e9 * LOG2E

F32 = jnp.float32
BF16 = jnp.bfloat16


def _dot(a, b):
    return jnp.dot(a, b, preferred_element_type=F32)


def _rows8(x):
    return [x[r:r + 8] for r in range(0, x.shape[0], 8)]


def _tree(op, xs):
    while len(xs) > 1:
        xs = [op(xs[i], xs[i + 1]) if i + 1 < len(xs) else xs[i] for i in range(0, len(xs), 2)]
    return xs[0]


def _all8(op, x):
    for sh in (4, 2, 1):
        x = op(x, pltpu.roll(x, sh, 0))
    return x


def _tile_rows(x, n):
    return jnp.concatenate([x] * n, axis=0)


def _layernorm(x):
    mean = _all8(jnp.add, _tree(jnp.add, _rows8(x))) * (1.0 / D)
    xc = x - _tile_rows(mean, D // 8)
    var = _all8(jnp.add, _tree(jnp.add, _rows8(xc * xc))) * (1.0 / D)
    return xc * _tile_rows(lax.rsqrt(var + EPS), D // 8)


def _local_block(q, k, v, k_prev, v_prev, first):
    lane = lax.broadcasted_iota(jnp.int32, k.shape, 1)

    def shifted(cur, prev, w):
        if w:
            cur = pltpu.roll(jnp.where(lane >= 128 - DIL * w, prev, cur), DIL * w, 1)
        return pltpu.bitcast(cur, BF16).astype(F32)

    logits = []
    for w in range(WIN):
        t = _all8(jnp.add, _tree(jnp.add, _rows8(q * shifted(k, k_prev, w))))
        if first and w:
            t = jnp.where(lane[:8] >= DIL * w, t, MASKED)
        logits.append(t)
    m = _tree(jnp.maximum, logits)
    p = [jnp.exp2(t - m) for t in logits]
    inv = 1.0 / _tree(jnp.add, p)
    o = None
    for w in range(WIN):
        t = shifted(v, v_prev, w) * _tile_rows(p[w], DH // 8)
        o = t if o is None else o + t
    return o * _tile_rows(inv, DH // 8)


def _kernel(x_hbm, aqkv_hbm, ao_hbm, bqkv_hbm, bo_hbm, out_hbm,
            io_ref, wraw_ref, woraw_ref, wt_ref, wot_ref, xt_ref, ht_ref,
            qt_ref, kn_ref, vt_ref, ot_ref, s_ref, m_ref, xsem, wsem, wosem):

    def x_copy(t):
        rows = pl.ds(t * BT, BT)
        return pltpu.make_async_copy(x_hbm.at[rows], io_ref.at[rows], xsem.at[t])

    def out_copy(t):
        rows = pl.ds(t * BT, BT)
        return pltpu.make_async_copy(io_ref.at[rows], out_hbm.at[rows], xsem.at[t])

    def w_copies(layer, g):
        src = (aqkv_hbm, bqkv_hbm)[layer]
        return [pltpu.make_async_copy(src.at[:, pl.ds(part * D + g * 128, 128)],
                                      wraw_ref.at[layer * NG + g, part], wsem.at[layer * NG + g])
                for part in range(3)]

    def w_wait(i):
        pltpu.make_async_copy(wraw_ref.at[i], wraw_ref.at[i], wsem.at[i]).wait()

    def wo_copy(layer):
        return pltpu.make_async_copy((ao_hbm, bo_hbm)[layer], woraw_ref.at[layer], wosem.at[layer])

    x_copy(0).start()
    for c in w_copies(0, 0):
        c.start()
    for t in range(1, NT):
        x_copy(t).start()
    for c in w_copies(0, 1):
        c.start()
    wo_copy(0).start()
    for layer in range(2):
        for g in range(2 if layer == 0 else 0, NG):
            for c in w_copies(layer, g):
                c.start()
    wo_copy(1).start()

    def prep_wqkv(i):
        for part in range(3):
            wt_ref[i, part * 128:(part + 1) * 128, :] = wraw_ref[i, part].T

    def prep_wo(layer, g):
        cols = pl.ds(pl.multiple_of(g * 128, 128), 128)
        wot_ref[layer, cols, :] = woraw_ref[layer, :, cols].T

    def load_block(t, carry):
        x_copy(t).wait()
        for u in range(BT // 128):
            rows = pl.ds(pl.multiple_of(t * BT + u * 128, 128), 128)
            x = io_ref[rows, :].T.astype(F32)
            xt_ref[t, :, u * 128:(u + 1) * 128] = x
            ht_ref[t, :, u * 128:(u + 1) * 128] = _layernorm(x).astype(BF16)
        return carry

    w_wait(0)
    prep_wqkv(0)
    lax.fori_loop(0, NT, load_block, 0)

    def qkv_local(rep):
        def body(g, carry):
            @pl.when(rep == 0)
            def _():
                w_wait(g + 1)

                @pl.when(g == 0)
                def _():
                    wo_copy(0).wait()

            w = wt_ref[g]
            for a in range(4):
                wa = jnp.concatenate([w[part * 128 + a * DH:part * 128 + (a + 1) * DH] for part in range(3)], axis=0)
                k_prev = v_prev = None
                for t in range(NT):
                    r = _dot(wa, ht_ref[t])
                    for u in range(BT // 128):
                        rr = r[:, u * 128:(u + 1) * 128]
                        k = pltpu.bitcast(rr[DH:2 * DH].astype(BF16), jnp.uint32)
                        v = pltpu.bitcast(rr[2 * DH:].astype(BF16), jnp.uint32)
                        first = t == 0 and u == 0
                        if first:
                            k_prev = k
                            v_prev = jnp.broadcast_to(v[:, :1], v.shape)
                        o = _local_block(rr[:DH] * QSCALE, k, v, k_prev, v_prev, first)
                        k_prev, v_prev = k, v
                        rows = pl.ds(pl.multiple_of(g * 128 + a * DH, DH), DH)
                        ot_ref[t, rows, u * 128:(u + 1) * 128] = o.astype(BF16)
            prep_wqkv(g + 1)
            prep_wo(0, g)
            return carry

        lax.fori_loop(0, NG, body, 0)

    def qkv_full(rep):
        def body(g, carry):
            nxt = jnp.minimum(NG + g + 1, 2 * NG - 1)

            @pl.when(rep == 0)
            def _():
                @pl.when(g < NG - 1)
                def _():
                    w_wait(nxt)

                @pl.when(g == 0)
                def _():
                    wo_copy(1).wait()

            w = wt_ref[NG + g]
            for t in range(NT):
                r = _dot(w, ht_ref[t])
                qt_ref[g * NT + t] = (r[:128] * QSCALE).astype(BF16)
                kn_ref[g, t * BT:(t + 1) * BT, :] = r[128:256].astype(BF16).T
                vt_ref[g, :, t * BT:(t + 1) * BT] = r[256:].astype(BF16)
            prep_wqkv(nxt)
            prep_wo(1, g)
            return carry

        lax.fori_loop(0, NG, body, 0)

    def attn_step(it_qk, it_pv, a):
        m = l = acc = None
        if it_qk is not None:
            g_qk = it_qk // NT
            q = qt_ref[it_qk, a * DH:(a + 1) * DH, :]
            zero = jnp.zeros_like(q)
            q = jnp.concatenate([q if b == a else zero for b in range(4)], axis=0)
        if it_pv is not None:
            g_pv = it_pv // NT
            m_pv = _tile_rows(m_ref[a], CK // 8)
        for c in range(S // CK):
            keys = slice(c * CK, (c + 1) * CK)
            if it_pv is not None:
                p = jnp.exp2(s_ref[a, keys, :] - m_pv)
                for slab in _rows8(p):
                    l = slab if l is None else l + slab
                p = p.astype(BF16)
            if it_qk is not None:
                s = _dot(kn_ref[g_qk, keys, :], q)
                s_ref[a, keys, :] = s
                for slab in _rows8(s):
                    m = slab if m is None else jnp.maximum(m, slab)
            if it_pv is not None:
                o = _dot(vt_ref[g_pv, a * DH:(a + 1) * DH, keys], p)
                acc = o if acc is None else acc + o
        if it_pv is not None:
            inv = 1.0 / _all8(jnp.add, l)
            rows = pl.ds(pl.multiple_of(g_pv * 128 + a * DH, DH), DH)
            ot_ref[it_pv % NT, rows, :] = (acc * _tile_rows(inv, DH // 8)).astype(BF16)
        if it_qk is not None:
            m_ref[a] = _all8(jnp.maximum, m)

    def attn_full():
        n_items = NG * NT
        for a in range(4):
            attn_step(0, None, a)

        def body(i, carry):
            for a in range(4):
                attn_step(i + 1, i, a)
            return carry

        lax.fori_loop(0, n_items - 1, body, 0)
        for a in range(4):
            attn_step(None, n_items - 1, a)

    def out_proj(layer):
        def body(t, carry):
            w = wot_ref[layer]
            for u in range(BT // 128):
                cols = slice(u * 128, (u + 1) * 128)
                x = xt_ref[t, :, cols] + _dot(w, ot_ref[t, :, cols])
                xt_ref[t, :, cols] = x
                ht_ref[t, :, cols] = _layernorm(x).astype(BF16)
            return carry

        lax.fori_loop(0, NT, body, 0)

    def out_proj_last(layer):
        def body(t, carry):
            w = wot_ref[layer]
            for u in range(BT // 128):
                cols = slice(u * 128, (u + 1) * 128)
                x = xt_ref[t, :, cols] + _dot(w, ot_ref[t, :, cols])
                rows = pl.ds(pl.multiple_of(t * BT + u * 128, 128), 128)
                io_ref[rows, :] = x.astype(BF16).T
            out_copy(t).start()
            return carry

        lax.fori_loop(0, NT, body, 0)

    def layer_pair(rep, carry):
        qkv_local(rep)
        out_proj(0)
        qkv_full(rep)
        attn_full()

        @pl.when(rep == 0)
        def _():
            out_proj(1)

        return carry

    lax.fori_loop(0, 2, layer_pair, 0)
    out_proj_last(1)
    for t in range(NT):
        out_copy(t).wait()


@jax.jit
def pallas_interleave_layers__sliding_local_dilated__softmax_full_mha__prompt_kernel(
    A_x: jax.Array,
    A_wqkv: jax.Array,
    A_wo: jax.Array,
    B_x: jax.Array,
    B_wqkv: jax.Array,
    B_wo: jax.Array,
):
    del B_x
    assert A_x.shape == (1, S, D)
    out = pl.pallas_call(
        _kernel,
        out_shape=jax.ShapeDtypeStruct((S, D), BF16),
        in_specs=[pl.BlockSpec(memory_space=pl.ANY)] * 5,
        out_specs=pl.BlockSpec(memory_space=pl.ANY),
        scratch_shapes=[
            pltpu.VMEM((S, D), BF16),
            pltpu.VMEM((2 * NG, 3, D, 128), BF16),
            pltpu.VMEM((2, D, D), BF16),
            pltpu.VMEM((2 * NG, 384, D), BF16),
            pltpu.VMEM((2, D, D), BF16),
            pltpu.VMEM((NT, D, BT), F32),
            pltpu.VMEM((NT, D, BT), BF16),
            pltpu.VMEM((NG * NT, 128, BT), BF16),
            pltpu.VMEM((NG, S, 128), BF16),
            pltpu.VMEM((NG, 128, S), BF16),
            pltpu.VMEM((NT, D, BT), BF16),
            pltpu.VMEM((4, S, BT), F32),
            pltpu.VMEM((4, 8, BT), F32),
            pltpu.SemaphoreType.DMA((NT,)),
            pltpu.SemaphoreType.DMA((2 * NG,)),
            pltpu.SemaphoreType.DMA((2,)),
        ],
        compiler_params=pltpu.CompilerParams(vmem_limit_bytes=112 * 1024 * 1024),
        name="interleaved_attention_layers",
    )(A_x.reshape(S, D), A_wqkv, A_wo, B_wqkv, B_wo)
    return out.reshape(1, S, D)
```

```python
import contextlib
import math

import jax
import jax.numpy as jnp
from jax import lax
import jax.experimental.pallas as pl
import jax.experimental.pallas.tpu as pltpu

S = 2048
D = 1024
H = 32
DH = D // H
WIN, DIL = 8, 2
EPS = 1e-5
NG = D // 128
NP = S // 256
BQ = 512
NQ = S // BQ
CK = 128
HD = D // 2
LOG2E = math.log2(math.e)
QSCALE = DH ** -0.5 * LOG2E
MASKED = -1e9 * LOG2E

STRASSEN = True
SCOPES = False
MC = 256
ONLY = None
LOCAL = "merge"
FLAGS = None
LAG = 11
NS = 4
OPAQUE = True
T0 = 16
TB = 10
WA = 30
WB = 24
WP = 28
WC = 14
WK = 14
WO = 24
ALINK = 1
NTR = 6
BURST = 1
LG = 2
IPB = 1
MSTEP = 2
C0 = 1
C1 = 3
MNUM = 1
MDEN = 1
W0 = (36, 30, 10)
REPS = (0, 1)
WN = 20

F32 = jnp.float32
BF16 = jnp.bfloat16
U32 = jnp.uint32


def _scheme():
    if STRASSEN:
        lhs = [[(1, 21), (-1, 11)], [(1, 12), (-1, 22)], [(1, 11), (1, 22)], [(1, 21), (1, 22)],
               [(1, 22)], [(1, 11)], [(1, 11), (1, 12)]]
        rhs = [[(1, 11), (1, 12)], [(1, 21), (1, 22)], [(1, 11), (1, 22)], [(1, 11)],
               [(1, 21), (-1, 11)], [(1, 12), (-1, 22)], [(1, 22)]]
        use = [[(1, 22)], [(1, 11)], [(1, 11), (1, 22)], [(1, 21), (-1, 22)],
               [(1, 11), (1, 21)], [(1, 12), (1, 22)], [(-1, 11), (1, 12)]]
        return lhs, rhs, [(i, i, use[i]) for i in range(7)]
    quads = [11, 12, 21, 22]
    ops = [[(1, q)] for q in quads]
    prods = [(quads.index(10 * i + k), quads.index(10 * k + j), [(1, 10 * i + j)])
             for j in (1, 2) for k in (1, 2) for i in (1, 2)]
    return ops, ops, prods


def _scope(name):
    return jax.named_scope(name) if SCOPES else contextlib.nullcontext()


def _dot(a, b):
    return jnp.dot(a, b, preferred_element_type=F32)


def _pack(x):
    return pltpu.bitcast(x.astype(BF16), U32)


def _put(ref, rows, cols, x):
    ref.bitcast(BF16)[rows, cols] = x.astype(BF16)


def _blk(i, n=128):
    return slice(i * n, (i + 1) * n)


def _bf16(x):
    return pltpu.bitcast(x, BF16)


def _combine(terms, quad):
    if len(terms) == 1:
        return quad[terms[0][1]]
    (_, a), (sign, b) = terms
    a, b = quad[a].astype(F32), quad[b].astype(F32)
    return a + b if sign > 0 else a - b


def _rows8(x):
    return [x[r:r + 8] for r in range(0, x.shape[0], 8)]


def _tree(op, xs):
    while len(xs) > 1:
        xs = [op(xs[i], xs[i + 1]) if i + 1 < len(xs) else xs[i] for i in range(0, len(xs), 2)]
    return xs[0]


def _all8(op, x):
    for sh in (4, 2, 1):
        x = op(x, pltpu.roll(x, sh, 0))
    return x


def _tile_rows(x, n):
    return jnp.concatenate([x] * n, axis=0)


def _tie(x, zero):
    if zero is None:
        return x
    return pltpu.bitcast(pltpu.bitcast(x, U32) | zero, x.dtype)


class _Pacer:
    def __init__(self, zero):
        self.zero = zero
        self.marks = []
        self.jobs = []
        self.due = {}

    def spread(self, jobs, first, last, window):
        for i, f in enumerate(jobs):
            due = first + (last - first) * i // max(len(jobs) - 1, 1)
            self.jobs.append((due - window, due, f))
        self.jobs.sort(key=lambda j: j[0])

    def block_product(self, lhs, rhs):
        out = {}
        for a, b, use in _scheme()[2]:
            now = len(self.marks)
            while self.jobs and self.jobs[0][0] < now:
                start, due, f = self.jobs.pop(0)
                self.due.setdefault(max(due, now), []).append(
                    f(pltpu.bitcast(self.marks[start], U32) & self.zero if start >= 0 else None))
            w = _rows8(lhs(a))
            for i, row in enumerate(w):
                if now + i in self.due:
                    w[i] = jnp.concatenate([row[:, :128] | _tree(jnp.bitwise_or, self.due[now + i]), row[:, 128:]], axis=1)
            m = _dot(_bf16(jnp.concatenate(w, axis=0)), _bf16(rhs(b)))
            self.marks += _rows8(m)[::2]
            for sign, q in use:
                out[q] = m if q not in out else (out[q] + m if sign > 0 else out[q] - m)
        return out


class _Stats:
    def __init__(self):
        self.x0 = self.s1 = self.s2 = None

    def add(self, x):
        for slab in _rows8(x):
            if self.x0 is None:
                self.x0 = slab
                continue
            d = slab - self.x0
            self.s1 = d if self.s1 is None else self.s1 + d
            self.s2 = d * d if self.s2 is None else self.s2 + d * d

    def finish(self):
        return self.finished(self.x0, self.s1, self.s2)

    @staticmethod
    def finished(x0, s1, s2):
        n = D // 8
        mean = _all8(jnp.add, x0 + s1 * (1.0 / n)) * 0.125
        e = x0 - mean
        var = _all8(jnp.add, s2 + e * (2.0 * s1 + n * e)) * (1.0 / D)
        return mean, lax.rsqrt(jnp.maximum(var, 0.0) + EPS)


def _shifted(cur, prev, w, lane):
    if w:
        cur = pltpu.roll(jnp.where(_tile_rows(lane, 2) >= 128 - DIL * w, prev, cur), DIL * w, 1)
    return _bf16(cur).astype(F32)


def _sum8(xs):
    row = lax.broadcasted_iota(jnp.int32, xs[0].shape, 0)
    for sh in (4, 2, 1):
        low = (row & sh) == 0
        if sh == 4:
            xs = [jnp.where(low, a, b) + pltpu.roll(jnp.where(low, b, a), 4, 0)
                  for a, b in zip(xs[:sh], xs[sh:])]
        else:
            xs = [jnp.where(low, a + pltpu.roll(a, 8 - sh, 0), b + pltpu.roll(b, sh, 0))
                  for a, b in zip(xs[:sh], xs[sh:])]
    return xs[0]


def _lanes(start):
    return _tie(lax.broadcasted_iota(jnp.int32, (8, 128), 1), start)


def _local_weights(q, k, k_prev, first, start):
    lane = _lanes(start)
    part = [_tree(jnp.add, _rows8(q * _shifted(k, k_prev, w, lane))) for w in range(WIN)]
    if LOCAL == "merge":
        t = _sum8(part)
        if first:
            t = jnp.where(lane >= DIL * lax.broadcasted_iota(jnp.int32, (8, 128), 0), t, MASKED)
        p = jnp.exp2(t - _all8(jnp.maximum, t))
        return [p / _all8(jnp.add, p)]
    logits = [_all8(jnp.add, t) for t in part]
    if first:
        logits = [jnp.where(lane >= DIL * w, t, MASKED) if w else t for w, t in enumerate(logits)]
    m = _tree(jnp.maximum, logits)
    p = [jnp.exp2(t - m) for t in logits]
    return p + [1.0 / _tree(jnp.add, p)]


def _local_values(p, v, v_prev, start):
    lane = _lanes(start)
    o = None
    for w in range(WIN):
        pw = jnp.broadcast_to(p[0][w:w + 1], (DH, 128)) if LOCAL == "merge" else _tile_rows(p[w], DH // 8)
        t = _shifted(v, v_prev, w, lane) * pw
        o = t if o is None else o + t
    return o if LOCAL == "merge" else o * _tile_rows(p[WIN], DH // 8)


def _kernel(x_hbm, aqkv_hbm, ao_hbm, bqkv_hbm, bo_hbm, out_hbm,
            io_ref, rawa_ref, rawb_ref, rawo_ref, wa_ref, wcur_ref, wb_ref, wo_ref, tr_refs, xa0_ref, xa1_ref, xb0_ref, xb1_ref, ht_ref, o_ref, ot_refs,
            qt_ref, kn_ref, vt_ref, s_refs, m_ref, lq_refs, lkv_refs, zero_ref, z_ref, xsem, wsem, rsem):
    lhs_ops, rhs_ops, nprod = _scheme()
    nprod = len(nprod)
    xa_ref, xb_ref = (xa0_ref, xa1_ref), (xb0_ref, xb1_ref)

    def x_copy(p):
        rows = pl.ds(p * 256, 256)
        return pltpu.make_async_copy(x_hbm.at[rows], io_ref.at[rows], xsem.at[p])

    def out_copy(p):
        rows = pl.ds(p * 256, 256)
        return pltpu.make_async_copy(io_ref.at[rows], out_hbm.at[rows], xsem.at[p])

    def cols(start):
        return pl.ds(start if isinstance(start, int) else pl.multiple_of(start, 128), 128)

    def start_qkv_a(g):
        for part in range(3):
            pltpu.make_async_copy(aqkv_hbm.at[:, cols(part * D + g * 128)], rawa_ref.at[g, part], wsem.at[g]).start()

    def wait_qkv_a(g):
        pltpu.make_async_copy(rawa_ref.at[g], rawa_ref.at[g], wsem.at[g]).wait()

    ao_copy = pltpu.make_async_copy(ao_hbm, rawo_ref.at[0], rsem.at[0])
    bo_copy = pltpu.make_async_copy(bo_hbm, rawo_ref.at[1], rsem.at[1])
    bqkv_copy = pltpu.make_async_copy(bqkv_hbm, rawb_ref, rsem.at[2])

    def prep_jobs(items):
        def transpose(buf, group):
            def run(start):
                for n, (tile, _, _) in enumerate(group):
                    for h in range(2):
                        t = tile(h)
                        if start is not None:
                            t = _bf16(pltpu.bitcast(t, U32) | _tile_rows(start, 8))
                        buf[0, 2 * n + h] = pltpu.bitcast(t.T, U32)
                return buf[z_ref[0], 2 * BURST, :8]
            return run

        def combine(buf, n, r, put, fence):
            def run(start):
                quad = {10 * (i + 1) + h + 1: _bf16(_tie(buf[z_ref[0], 2 * n + h, _blk(4 * i + r, 8)], start))
                        for i in range(2) for h in range(2)}
                for i, terms in enumerate(lhs_ops):
                    put(i, r, _combine(terms, quad))
                return fence()
            return run
        out = []
        for j in range(0, len(items), BURST):
            buf, group = tr_refs[j // BURST % len(tr_refs)], items[j:j + BURST]
            out.append((transpose(buf, group),
                        [combine(buf, n, r, put, fence) for n, (_, put, fence) in enumerate(group) for r in range(4)]))
        return out

    def pace_prep(pacer, items, first, last):
        jobs = prep_jobs(items)
        step = (last - first - WC) // len(jobs)
        for j, (a, b) in enumerate(jobs):
            pacer.spread([a], first + j * step, first + j * step, WP)
            pacer.spread(b, first + j * step + WC, first + (j + 1) * step + WC, WC)

    def qkv_items(g, layer, dst_ref, k):
        def tile(part, r):
            return rawb_ref[_blk(r), cols(part * D + g * 128)] if layer else rawa_ref[g, part, _blk(r), :]
        return [(lambda h, part=part, c=c: tile(part, 4 * h + c),
                 lambda i, r, x, part=part, c=c: _put(dst_ref.at[k, i], _blk(4 * (1, 0, 2)[part] + r, 16), _blk(c), x),
                 lambda: dst_ref[z_ref[0], 0, 96:, :128]) for part in range(3) for c in range(4)]

    def wo_items(layer, g):
        def tile(c, h):
            return jnp.concatenate([rawo_ref[layer, _blk(4 * c + h + 2 * i, 64), cols(g * 128)] for i in range(2)], axis=0)
        return [(lambda h, c=c: tile(c, h),
                 lambda i, r, x, c=c: _put(wo_ref.at[layer, i], pl.ds(pl.multiple_of(g * 64 + r * 16, 16), 16), _blk(c), x),
                 lambda: wo_ref[z_ref[0], 0, HD // 2:, :128]) for c in range(4)]

    def normalize_jobs(x_ref, p, stats, n):
        def job(rows):
            def run(start):
                (m1, r1), (m2, r2) = [(_tile_rows(_tie(m, start), 2), _tile_rows(r, 2)) for m, r in stats()]
                for r in rows:
                    quad = {11: (x_ref[0, r:r + 16] - m1) * r1,
                            12: (x_ref[1, r:r + 16] - m2) * r2,
                            21: (x_ref[0, HD + r:HD + r + 16] - m1) * r1,
                            22: (x_ref[1, HD + r:HD + r + 16] - m2) * r2}
                    for i, terms in enumerate(rhs_ops):
                        _put(ht_ref.at[p], slice(r, r + 16), _blk(i), _combine(terms, quad))
                return ht_ref[0, HD // 2:, :128]
            return run
        step = HD // n
        return [job(range(i * step, (i + 1) * step, 16)) for i in range(n)]

    def layernorm_jobs(x_ref, p):
        sts = [_Stats(), _Stats()]
        done = []

        def measure(c):
            def run(start):
                for b in range(2):
                    if sts[b].x0 is not None:
                        sts[b].x0 = _tie(sts[b].x0, start)
                    sts[b].add(x_ref[b, _blk(c)])
                return _tree(jnp.bitwise_or, [pltpu.bitcast(v, U32) for st in sts for v in (st.s1, st.s2)]) & zero()
            return run

        def stats():
            if not done:
                done.extend(st.finish() for st in sts)
            return done
        return [measure(c) for c in range(NG)] + normalize_jobs(x_ref, p, stats, 16)

    def operand_jobs(p, slot, normalize):
        def job(g, c):
            def run(start):
                quad = {}
                for i in range(2):
                    for b in range(2):
                        src = o_ref.at[2 * p + b, 4 * g + 2 * i + c]
                        if normalize:
                            o = src[:DH] * _tile_rows(1.0 / _all8(jnp.add, _tie(src[DH:], start)), DH // 8)
                        else:
                            o = _tie(src[:DH], None if start is None else _tile_rows(start, DH // 8))
                        quad[10 * (i + 1) + b + 1] = o
                for i, terms in enumerate(rhs_ops):
                    _put(ot_refs[slot].at[z_ref[0]], _blk(2 * g + c, DH), _blk(i), _combine(terms, quad))
                return ot_refs[slot][0, HD // 2:, :128]
            return run
        return [job(g, c) for g in range(NG) for c in range(2)]

    def zero():
        return zero_ref[...]

    def load_pairs(t, carry):
        for pp in range(2):
            p = 2 * t + pp
            x_copy(p).wait()

            @pl.when(p + 2 < NP)
            def _():
                x_copy(p + 2).start()

            if pp == 0:
                @pl.when(p == NP - 4)
                def _():
                    start_qkv_a(0)

            stats = []
            for b in range(2):
                rows = pl.ds(pl.multiple_of(p * 256 + b * 128, 128), 128)
                st = _Stats()
                for c in range(NG):
                    x = io_ref[rows, c * 128:(c + 1) * 128].T.astype(F32)
                    xa_ref[pp][t, b, c * 128:(c + 1) * 128] = x
                    st.add(x)
                stats.append(st.finish())
            for f in normalize_jobs(xa_ref[pp].at[t], p, lambda: stats, 1):
                f(None)
        return carry

    with _scope("pro"):
        x_copy(0).start()
        x_copy(1).start()
        for ref in tr_refs:
            ref[0, 2 * BURST, :8] = jnp.zeros((8, 128), U32)
        for ref in lq_refs[-2:] + lkv_refs[-3:]:
            ref[...] = jnp.zeros(ref.shape, ref.dtype)
        z_ref[0] = 0
        zs = jnp.zeros((8, 128), U32)
        zero_ref[...] = zs
        ht_ref[0, HD // 2:, :128] = zs
        o_ref[0, H, :8] = jnp.zeros((8, 128), F32)
        for ref in ot_refs:
            ref[0, HD // 2:, :128] = zs
        wo_ref[0, 0, HD // 2:, :128] = zs
        for ref in (wa_ref, wcur_ref, wb_ref):
            ref[0, 0, 96:, :128] = zs
        lax.fori_loop(0, NP // 2, load_pairs, 0)
        start_qkv_a(1)
        wait_qkv_a(0)
        ao_copy.start()
        jobs = prep_jobs(qkv_items(0, 0, wa_ref, 0))
        jobs[0][0](None)
        for n, (_, b) in enumerate(jobs):
            for f in [a for a, _ in jobs[n + 1:n + 2]] + b:
                f(None)
        wcur_ref[0, :, :96] = wa_ref[0, :, :96]

    z = z_ref[0]

    def staged(refs, u):
        return refs[u // 2 % NS].at[u % 2 + (z if OPAQUE else 0)]

    def local_jobs(g):
        weights = {}

        def first_step(u, a):
            def run(start):
                head = _blk(a, DH // 2)
                k = staged(lkv_refs, u)[head, :128]
                k_prev = staged(lkv_refs, u - 1)[head, :128] if u else k
                p = weights[u, a] = _local_weights(staged(lq_refs, u)[_blk(a, DH)], k, k_prev, u == 0, start)
                return pltpu.bitcast(p[-1], U32) & zero()
            return run

        def second_step(u, a):
            def run(start):
                head = _blk(a, DH // 2)
                v = staged(lkv_refs, u)[head, 128:]
                v_prev = staged(lkv_refs, u - 1)[head, 128:] if u else jnp.broadcast_to(v[:, :1], v.shape)
                o_ref[u, 4 * g + a, :DH] = _local_values(weights[u, a], v, v_prev, start)
                return pltpu.bitcast(o_ref[0, H, :8], U32)
            return run
        units = [(2 * p + b, a) for p in range(NP) for a in (2, 3, 0, 1) for b in range(2)]
        return [first_step(*k) for k in units], [second_step(*k) for k in units]

    def qkv_local(rep):
        def body(g, prepare):
            pacer = _Pacer(zero())
            ticks = NP * nprod * 12
            (a0, b0), (a1, b1) = local_jobs(jnp.maximum(g - 1, 0)), local_jobs(g)
            wa, wb, tb = W0 if prepare else (WA, WB, TB)
            pacer.spread(a0[-LAG:] + a1[:-LAG], T0, ticks - 1 - tb, wa)
            pacer.spread(b0[-LAG:] + b1[:-LAG], T0 + tb, ticks - 1, wb)
            nxt = (g + 1) % NG
            if prepare:
                @pl.when(g + 1 < NG)
                def _():
                    wait_qkv_a(g + 1)

                @pl.when(g + 2 < NG)
                def _():
                    start_qkv_a(g + 2)

                @pl.when(g == 0)
                def _():
                    ao_copy.wait()

                @pl.when(g == NG - 2)
                def _():
                    bqkv_copy.start()
                    bo_copy.start()

                pace_prep(pacer, qkv_items(nxt, 0, wa_ref, nxt) + wo_items(0, g), WP, ticks - 1)

                def copy(i, r):
                    def run(start):
                        wcur_ref[z, i, _blk(r, 24)] = wa_ref[nxt + z, i, _blk(r, 24)] | jnp.tile(start, (3, 4))
                        return wcur_ref[0, 0, 96:, :128]
                    return run
                pacer.spread([copy(i, r) for i in range(len(lhs_ops)) for r in range(4)],
                             ticks - nprod * 12 + WK, ticks - 1, WK)

            def lhs(p, i):
                return wcur_ref[0, i, :96] if prepare and p < NP - 1 else wa_ref[g, i, :96]

            for p in range(NP):
                r = pacer.block_product(lambda i: lhs(p, i), lambda i: ht_ref[p, :HD // 2, _blk(i)])
                for i, b in ((1, 0), (1, 1), (0, 0), (0, 1)):
                    rr = r[10 * (i + 1) + b + 1]
                    _put(lkv_refs[p % NS].at[b], _blk(i, 64), _blk(0), rr[:64])
                    lq_refs[p % NS][b, _blk(i, 64)] = rr[64:128] * QSCALE
                    _put(lkv_refs[p % NS].at[b], _blk(i, 64), _blk(1), rr[128:])
            assert not pacer.jobs

        pl.loop(0, NG)(lambda g: body(g, rep == 0))

        a1, b1 = [jobs[-LAG:] for jobs in local_jobs(NG - 1)]
        for f in operand_jobs(0, 0, False):
            f(None)
        a1[0](None)
        for i in range(LAG):
            for f in a1[i + 1:i + 2] + b1[i:i + 1]:
                f(None)

    def qkv_full(rep):
        def body(g, carry):
            pacer = _Pacer(zero())
            if rep == 0:
                pace_prep(pacer, wo_items(1, g), 5 * 12, (4 * nprod + 5) * 12 + WC)
            for p in range(NP):
                r = pacer.block_product(lambda i: wb_ref[g, i, :96], lambda i: ht_ref[p, :HD // 2, _blk(i)])
                for b in range(2):
                    u = 2 * p + b
                    k, q, v = [jnp.concatenate([r[11 + b][part * 64:(part + 1) * 64],
                                                r[21 + b][part * 64:(part + 1) * 64]], axis=0) for part in range(3)]
                    _put(qt_ref.at[g * NQ + u // 4], slice(None), slice((u % 4) * 128, (u % 4 + 1) * 128), q * QSCALE)
                    kn_ref[g, _blk(u, 64), :] = pltpu.bitcast(k.astype(BF16).T, U32)
                    _put(vt_ref.at[g], slice(None), slice(u * 128, (u + 1) * 128), v)
            return carry

        lax.fori_loop(0, NG, body, 0)

    def attn_step(qk, pv, slot, m_pv, marks, leftover, l_prev, acc_prev):
        m = l = acc = None
        wide_zero = jnp.concatenate([zero()] * (BQ // 128), axis=1)
        if qk is not None:
            g_qk = qk[0] // NQ
            q = _bf16(qt_ref[qk[0], _blk(qk[1], DH // 2), :])
            blank = jnp.zeros_like(q)
            q = jnp.concatenate([q if b == qk[1] else blank for b in range(4)], axis=0)
        if pv is not None:
            g_pv = pv[0] // NQ
        for c in range(S // CK):
            if c == C0 and leftover:
                done = leftover(pltpu.bitcast(marks[0], U32) & wide_zero if marks else None)
            if c == C1 and leftover and pv is not None:
                m_pv = _tie(m_pv, done & wide_zero)
            if pv is not None:
                p = []
                for i in range(CK // 16):
                    if i % MSTEP == 0:
                        top = _tie(m_pv, pltpu.bitcast(marks[i * MNUM // MDEN], U32) & wide_zero) if marks else m_pv
                    e = jnp.exp2(s_refs[slot][c + z, _blk(CK // 16 - 1 - i, 16)] - _tile_rows(top, 2))
                    if l is None:
                        l = _tie(e[:8] + e[8:], None if l_prev is None else pltpu.bitcast(l_prev, U32) & wide_zero)
                    else:
                        l = l + (e[:8] + e[8:])
                    p.append(e)
                p = jnp.concatenate(p[::-1], axis=0).astype(BF16)
            link = pltpu.bitcast(marks[-1], U32) & wide_zero if marks else None
            del marks[:]
            if qk is not None:
                s = _dot(_bf16(kn_ref[g_qk, _blk(c, CK // 2), :]), q)
                s_refs[(slot + LG) % 4][c] = s
                for i, slab in enumerate(_rows8(s)):
                    m = _tie(slab, link) if m is None else jnp.maximum(m, slab)
                    if i % 2:
                        marks.append(m)
            if pv is not None:
                o = _dot(_bf16(vt_ref[g_pv, _blk(pv[1], DH // 2), _blk(c, CK)]), p)
                if acc is None:
                    acc = _tie(o, pltpu.bitcast(acc_prev, U32) & _tile_rows(wide_zero, DH // 8) if ALINK and acc_prev is not None else None)
                else:
                    acc = acc + o
        return m, l, acc

    def attn_steps(item, first, last, n_steps):
        def head(n):
            return (item + n // 4, n % 4) if 0 <= n < n_steps else None
        tops, marks = {}, []

        def finish(n, m):
            def run(start):
                tops[n % LG] = _all8(jnp.maximum, _tie(m, start))
                return pltpu.bitcast(tops[n % LG], U32)
            return run

        leftover = l = acc = None
        for n in range(first, last):
            m_pv = None if n < 0 else tops[n % LG] if n % LG in tops else m_ref[n % LG]
            m, l, acc = attn_step(head(n + LG), head(n), n % 4, m_pv, marks, leftover, l, acc)
            if l is not None:
                it, a = head(n)
                for j in range(BQ // 128):
                    o_ref[(it % NQ) * (BQ // 128) + j, (it // NQ) * 4 + a] = jnp.concatenate([acc, l], axis=0)[:, _blk(j)]
            leftover = None
            if m is not None and LG == 1:
                finish(n, m)(None)
            elif m is not None:
                leftover = finish(n, m)
        if leftover:
            leftover(None)
        for slot, val in tops.items():
            m_ref[slot] = val

    def attn_full():
        n_items = NG * NQ
        trips = (n_items - 1) // IPB
        lead = n_items - 1 - trips * IPB
        attn_steps(0, -LG, 4 * lead, 4 * n_items)

        def body(i, carry):
            attn_steps(lead + i * IPB, 0, 4 * IPB, 4 * n_items)
            return carry

        with _scope("attn_loop"):
            lax.fori_loop(0, trips, body, 0)
        for f in operand_jobs(0, 0, True):
            f(None)
        attn_steps(n_items - 1, 0, 4, 4)

    def project_pair(pacer, layer, src_ref, slot, emit):
        n = HD // MC
        for j in range(n):
            r = pacer.block_product(lambda i: wo_ref[layer, i, j * MC // 2:(j + 1) * MC // 2, :],
                                    lambda i: ot_refs[slot][0, :HD // 2, _blk(i)])
            for c in range(MC // 64):
                f = (j * (MC // 64) + c) * 128
                for b in range(2):
                    y = jnp.concatenate([r[11 + b][c * 64:(c + 1) * 64], r[21 + b][c * 64:(c + 1) * 64]], axis=0)
                    emit(b, f, src_ref[b, f:f + 128] + y)

    def operand_pacer(layer, t):
        pacer = _Pacer(zero())
        ticks = nprod * HD // 16
        pacer.spread(operand_jobs(2 * t + 1, 1, layer == 1), WO, ticks - WO, WO)
        pacer.spread(operand_jobs(jnp.minimum(2 * t + 2, NP - 1), 0, layer == 1), ticks + WO, 2 * ticks - 1, WO)
        return pacer, ticks

    def out_proj(layer, src_ref, dst_ref, prepare):
        def body(t, carry):
            pacer, ticks = operand_pacer(layer, t)
            last = jnp.maximum(t - 1, 0)
            pacer.spread(layernorm_jobs(dst_ref[1].at[last], 2 * last + 1), WN, ticks - 1, WN)
            pacer.spread(layernorm_jobs(dst_ref[0].at[t], 2 * t), ticks + WN, 2 * ticks - 1, WN)
            if prepare:
                pace_prep(pacer, qkv_items(2 * t, 1, wb_ref, 2 * t) + qkv_items(2 * t + 1, 1, wb_ref, 2 * t + 1),
                          WP, 2 * ticks - 1)
            for pp in range(2):
                def emit(b, f, x):
                    dst_ref[pp][t, b, f:f + 128] = x

                project_pair(pacer, layer, src_ref[pp].at[t], pp, emit)
            return carry

        lax.fori_loop(0, NP // 2, body, 0)
        for f in layernorm_jobs(dst_ref[1].at[NP // 2 - 1], NP - 1):
            f(None)

    def out_proj_last(layer, src_ref):
        def body(t, carry):
            pacer, _ = operand_pacer(layer, t)
            for pp in range(2):
                p = 2 * t + pp

                def emit(b, f, x):
                    rows = pl.ds(pl.multiple_of(p * 256 + b * 128, 128), 128)
                    io_ref[rows, f:f + 128] = x.astype(BF16).T

                project_pair(pacer, layer, src_ref[pp].at[t], pp, emit)
                out_copy(p).start()
            return carry

        lax.fori_loop(0, NP // 2, body, 0)

    def layer_pair(rep, carry):
        if ONLY in (None, "local"):
            with _scope("qkv_local"):
                qkv_local(rep)
        if rep == 0:
            bqkv_copy.wait()
            bo_copy.wait()

        if ONLY in (None, "out"):
            with _scope("out0"):
                out_proj(0, xa_ref, xb_ref, rep == 0)
        if ONLY in (None, "full", "out"):
            with _scope("qkv_full"):
                qkv_full(rep)
        if ONLY in (None, "attn", "full"):
            attn_full()

        if rep == 0:
            if ONLY in (None, "out"):
                with _scope("out1"):
                    out_proj(1, xb_ref, xa_ref, False)

        return carry

    xb1_ref[0] = jnp.zeros(xb1_ref.shape[1:], F32)
    for rep in REPS:
        layer_pair(rep, 0)
    with _scope("last"):
        out_proj_last(1, xb_ref)
    for p in range(NP):
        out_copy(p).wait()


@jax.jit
def pallas_interleave_layers__sliding_local_dilated__softmax_full_mha__prompt_kernel(
    A_x: jax.Array,
    A_wqkv: jax.Array,
    A_wo: jax.Array,
    B_x: jax.Array,
    B_wqkv: jax.Array,
    B_wo: jax.Array,
):
    del B_x
    assert A_x.shape == (1, S, D)
    nb = len(_scheme()[0])
    out = pl.pallas_call(
        _kernel,
        out_shape=jax.ShapeDtypeStruct((S, D), BF16),
        in_specs=[pl.BlockSpec(memory_space=pl.ANY)] * 5,
        out_specs=pl.BlockSpec(memory_space=pl.ANY),
        scratch_shapes=[
            pltpu.VMEM((S, D), BF16),
            pltpu.VMEM((NG, 3, D, 128), BF16),
            pltpu.VMEM((D, 3 * D), BF16),
            pltpu.VMEM((2, D, D), BF16),
            pltpu.VMEM((NG, nb, 96 + 8, HD), U32),
            pltpu.VMEM((1, nb, 96 + 8, HD), U32),
            pltpu.VMEM((NG, nb, 96 + 8, HD), U32),
            pltpu.VMEM((2, nb, HD // 2 + 8, HD), U32),
            [pltpu.VMEM((1, 2 * BURST + 1, 64, 128), U32)] * NTR,
            *[pltpu.VMEM((NP // 2, 2, D, 128), F32)] * 4,
            pltpu.VMEM((NP, HD // 2 + 8, nb * 128), U32),
            pltpu.VMEM((2 * NP, H + 1, DH + 8, 128), F32),
            [pltpu.VMEM((1, HD // 2 + 8, nb * 128), U32)] * 2,
            pltpu.VMEM((NG * NQ, 64, BQ), U32),
            pltpu.VMEM((NG, S // 2, 128), U32),
            pltpu.VMEM((NG, 64, S), U32),
            [pltpu.VMEM((S // CK, CK, BQ), F32)] * 4,
            pltpu.VMEM((4, 8, BQ), F32),
            [pltpu.VMEM((2, 128, 128), F32)] * NS,
            [pltpu.VMEM((2, 64, 256), U32)] * NS,
            pltpu.VMEM((8, 128), U32),
            pltpu.SMEM((1,), jnp.int32),
            pltpu.SemaphoreType.DMA((NP,)),
            pltpu.SemaphoreType.DMA((NG,)),
            pltpu.SemaphoreType.DMA((3,)),
        ],
        compiler_params=pltpu.CompilerParams(vmem_limit_bytes=120 * 1024 * 1024, flags=FLAGS),
        name="interleaved_attention_layers",
    )(A_x.reshape(S, D), A_wqkv, A_wo, B_wqkv, B_wo)
    return out.reshape(1, S, D)
```

```python
import math

import jax
import jax.numpy as jnp
from jax import lax
import jax.experimental.pallas as pl
import jax.experimental.pallas.tpu as pltpu

S = 2048
D = 1024
H = 32
DH = D // H
WIN, DIL = 8, 2
EPS = 1e-5
LOG2E = math.log2(math.e)
QSCALE = DH ** -0.5 * LOG2E
MASKED = -1e9 * LOG2E

HD = D // 2
NG = D // 128
NP = S // 256
MQ = 192
MO = 256
BQ = 512
NQ = S // BQ
CK = 128
NC = S // CK

NS = 4
NTR = 6
LAG = 11
SKEW = 2
IPB = 2
GPB = 2

W_LOCAL = ((36, 30), (30, 24), (34, 28))
W_XPOSE, W_COMBINE, W_NORM, W_OPERAND, W_VALUES = 28, 14, 20, 20, 26

F32 = jnp.float32
BF16 = jnp.bfloat16
U32 = jnp.uint32

LHS = (((1, 21), (-1, 11)), ((1, 12), (-1, 22)), ((1, 11), (1, 22)), ((1, 21), (1, 22)),
       ((1, 22),), ((1, 11),), ((1, 11), (1, 12)))
RHS = (((1, 11), (1, 12)), ((1, 21), (1, 22)), ((1, 11), (1, 22)), ((1, 11),),
       ((1, 21), (-1, 11)), ((1, 12), (-1, 22)), ((1, 22),))
USE = (((1, 22),), ((1, 11),), ((1, 11), (1, 22)), ((1, 21), (-1, 22)),
       ((1, 11), (1, 21)), ((1, 12), (1, 22)), ((-1, 11), (1, 12)))
NB = len(USE)


def _blk(i, n=128):
    return slice(i * n, (i + 1) * n) if isinstance(i, int) else pl.ds(pl.multiple_of(i * n, n), n)


def _dot(a, b):
    return jnp.dot(a, b, preferred_element_type=F32)


def _bits(x):
    return pltpu.bitcast(x, U32)


def _bf16(x):
    return pltpu.bitcast(x, BF16)


def _put(ref, rows, cols, x):
    ref.bitcast(BF16)[rows, cols] = x.astype(BF16)


def _combine(terms, blocks):
    if len(terms) == 1:
        return blocks[terms[0][1]]
    (_, a), (sign, b) = terms
    a, b = blocks[a].astype(F32), blocks[b].astype(F32)
    return a + b if sign > 0 else a - b


def _rows8(x):
    return [x[r:r + 8] for r in range(0, x.shape[0], 8)]


def _tile(x, rows, cols=1):
    if cols > 1:
        x = jnp.concatenate([x] * cols, axis=1)
    return jnp.concatenate([x] * rows, axis=0) if rows > 1 else x


def _tree(op, xs):
    while len(xs) > 1:
        xs = [op(xs[i], xs[i + 1]) if i + 1 < len(xs) else xs[i] for i in range(0, len(xs), 2)]
    return xs[0]


def _all8(op, x):
    for sh in (4, 2, 1):
        x = op(x, pltpu.roll(x, sh, 0))
    return x


def _sum8(xs):
    row = lax.broadcasted_iota(jnp.int32, xs[0].shape, 0)
    low = (row & 4) == 0
    xs = [jnp.where(low, a, b) + pltpu.roll(jnp.where(low, b, a), 4, 0) for a, b in zip(xs[:4], xs[4:])]
    for sh in (2, 1):
        low = (row & sh) == 0
        xs = [jnp.where(low, a + pltpu.roll(a, 8 - sh, 0), b + pltpu.roll(b, sh, 0))
              for a, b in zip(xs[:sh], xs[sh:])]
    return xs[0]


def _after(x, token):
    if token is None:
        return x
    token = _tile(token, x.shape[0] // token.shape[0], x.shape[1] // token.shape[1])
    return pltpu.bitcast(_bits(x) | token, x.dtype)


def _fence(ref, z=0):
    return _bits(ref[(z,) + (0,) * (len(ref.shape) - 3) + (slice(ref.shape[-2] - 8, None), _blk(0))])


class _Pacer:
    def __init__(self, zero):
        self.zero = zero
        self.marks = []
        self.jobs = []
        self.due = {}

    def spread(self, jobs, first, last, window):
        for i, job in enumerate(jobs):
            due = first + (last - first) * i // max(len(jobs) - 1, 1)
            self.jobs.append((due - window, due, job))
        self.jobs.sort(key=lambda j: j[0])

    def flush(self):
        now = len(self.marks)
        while self.jobs and self.jobs[0][0] < now:
            start, due, job = self.jobs.pop(0)
            done = job(_bits(self.marks[start]) & self.zero if start >= 0 else None)
            self.due.setdefault(max(due, now), []).append(done)

    def block_product(self, lhs, rhs):
        out = {}
        for i, use in enumerate(USE):
            self.flush()
            now = len(self.marks)
            w = _rows8(lhs(i))
            for j, row in enumerate(w):
                if now + j in self.due:
                    w[j] = jnp.concatenate(
                        [row[:, :128] | _tree(jnp.bitwise_or, self.due[now + j]), row[:, 128:]], axis=1)
            m = _dot(_bf16(jnp.concatenate(w, axis=0)), _bf16(rhs(i)))
            self.marks += [m[16 * j:16 * j + 8] for j in range(len(w))]
            for sign, b in use:
                out[b] = m if b not in out else (out[b] + m if sign > 0 else out[b] - m)
        return out


class _Moments:
    def __init__(self):
        self.x0 = self.s1 = self.s2 = None

    def add(self, x):
        for slab in _rows8(x):
            if self.x0 is None:
                self.x0 = slab
                continue
            d = slab - self.x0
            self.s1 = d if self.s1 is None else self.s1 + d
            self.s2 = d * d if self.s2 is None else self.s2 + d * d

    def mean_and_scale(self):
        n = D // 8
        mean = _all8(jnp.add, self.x0 + self.s1 * (1.0 / n)) * 0.125
        e = self.x0 - mean
        var = _all8(jnp.add, self.s2 + e * (2.0 * self.s1 + n * e)) * (1.0 / D)
        return mean, lax.rsqrt(jnp.maximum(var, 0.0) + EPS)


def _window_slot(cur, prev, w, lane):
    if w:
        cur = pltpu.roll(jnp.where(_tile(lane, 2) >= 128 - DIL * w, prev, cur), DIL * w, 1)
    return _bf16(cur).astype(F32)


def _exp_scores(scores, tops, total, link):
    p = []
    for i in range(CK // 16):
        e = jnp.exp2(scores(_blk(CK // 16 - 1 - i, 16)) - _tile(tops[i], 2))
        total = _after(e[:8] + e[8:], link) if total is None else total + (e[:8] + e[8:])
        p.append(e)
    return jnp.concatenate(p[::-1], axis=0).astype(BF16), total


def _kernel(x_hbm, aqkv_hbm, ao_hbm, bqkv_hbm, bo_hbm, out_hbm,
            io_ref, rawa_ref, rawb_ref, rawo_ref, tr_refs, wa_ref, wcur_ref, wb_ref, wo_ref,
            xa_refs, xb_refs, h_refs, o_ref, op_refs, lq_refs, lkv_refs,
            q_ref, k_ref, v_ref, s_refs, m_ref, zero_ref, z_ref, xsem, asem, bsem):

    def zero():
        return zero_ref[...]

    def z():
        return z_ref[0]

    def token(*values):
        return _tree(jnp.bitwise_or, [_bits(v) for v in values]) & _tile(zero(), 1, values[0].shape[1] // 128)

    arrived = set()

    def x_copy(p):
        return pltpu.make_async_copy(x_hbm.at[_blk(p, 256)], io_ref.at[_blk(p, 256)], xsem.at[p])

    def out_copy(p):
        return pltpu.make_async_copy(io_ref.at[_blk(p, 256)], out_hbm.at[_blk(p, 256)], xsem.at[p])

    def start_local_weights(g):
        srcs = [aqkv_hbm.at[:, _blk(part * NG + g)] for part in range(3)] + [ao_hbm.at[:, _blk(g)]]
        for i, src in enumerate(srcs):
            pltpu.make_async_copy(src, rawa_ref.at[g, i], asem.at[g]).start()

    def wait_local_weights(g):
        pltpu.make_async_copy(rawa_ref.at[g], rawa_ref.at[g], asem.at[g]).wait()
        if isinstance(g, int):
            arrived.add(("w", g))

    def wait_input(p):
        x_copy(p).wait()
        arrived.add(("x", p))

    def full_weight_copies(rows):
        return [pltpu.make_async_copy(src.at[rows], dst.at[rows], bsem.at[i])
                for i, (src, dst) in enumerate(((bqkv_hbm, rawb_ref), (bo_hbm, rawo_ref)))]

    staged_tiles = {}
    n_tiles = [0]

    def weight_jobs(tile, dst_ref, index, row, c):
        slot = n_tiles[0] % NTR
        n_tiles[0] += 1
        buf = tr_refs[slot]

        def transpose(start):
            staged_tiles[slot] = tile
            for h in range(2):
                t = tile(h) if start is None else _bf16(_after(_bits(tile(h)), start))
                buf[0, h, :64] = _bits(t.T)
            return _fence(buf, z())

        def combine(r):
            def run(start):
                assert staged_tiles[slot] is tile
                blocks = {10 * i + h + 11: _bf16(_after(buf[z(), h, _blk(4 * i + r, 8)], start))
                          for i in range(2) for h in range(2)}
                for i, terms in enumerate(LHS):
                    _put(dst_ref.at[index, i], _blk(row + r, 16), _blk(c), _combine(terms, blocks))
                return _fence(dst_ref, z())
            return run
        return transpose, [combine(r) for r in range(4)]

    def qkv_weight_jobs(layer, g, first_ref=None):
        def tile(part, r):
            assert layer or not isinstance(g, int) or ("w", g) in arrived
            return rawb_ref[_blk(r), _blk(part * NG + g)] if layer else rawa_ref[g, part, _blk(r), :]
        return [weight_jobs(lambda h, part=part, c=c: tile(part, 4 * h + c),
                            (wb_ref if layer else wa_ref) if first_ref is None else first_ref, g, 4 * (1, 0, 2)[part], c)
                for part in range(3) for c in range(4)]

    def out_weight_jobs(layer, g):
        def rows(r):
            return rawo_ref[_blk(r, 64), _blk(g)] if layer else rawa_ref[g, 3, _blk(r, 64), :]
        return [weight_jobs(lambda h, c=c: jnp.concatenate([rows(4 * c + h), rows(4 * c + h + 2)], axis=0),
                            wo_ref, layer, 4 * g, c) for c in range(4)]

    def pace_weights(pacer, jobs, first, last):
        step = (last - first - W_COMBINE) // len(jobs)
        for j, (transpose, combine) in enumerate(jobs):
            t = first + j * step
            pacer.spread([transpose], t, t, W_XPOSE)
            pacer.spread(combine, t + W_COMBINE, t + step + W_COMBINE, W_COMBINE)

    def h_operand(p, fresh):
        src = h_refs[p % 2].at[p // 2 + (z() if fresh else 0)]
        return lambda i: src[:HD // 2, _blk(i)]

    def normalize_jobs(x_ref, dst_ref, index, stats):
        def job(j):
            def run(start):
                st = [(_tile(_after(mean, start), 2), _tile(scale, 2)) for mean, scale in stats()]
                for r in (2 * j, 2 * j + 1):
                    blocks = {10 * h + b + 11: (x_ref[b, _blk(h * HD // 16 + r, 16)] - st[b][0]) * st[b][1]
                              for h in range(2) for b in range(2)}
                    for i, terms in enumerate(RHS):
                        _put(dst_ref.at[index], _blk(r, 16), _blk(i), _combine(terms, blocks))
                return _fence(dst_ref, z())
            return run
        return [job(j) for j in range(HD // 32)]

    def layernorm_jobs(x_ref, dst_ref, index):
        moments, done = [_Moments(), _Moments()], []

        def measure(c):
            def run(start):
                for b, mo in enumerate(moments):
                    if mo.x0 is not None:
                        mo.x0 = _after(mo.x0, start)
                    mo.add(x_ref[b, _blk(c)])
                return token(*[v for mo in moments for v in (mo.s1, mo.s2)])
            return run

        def stats():
            if not done:
                done.extend(mo.mean_and_scale() for mo in moments)
            return done
        return [measure(c) for c in range(NG)] + normalize_jobs(x_ref, dst_ref, index, stats)

    def last_layernorm_jobs(x_refs):
        return layernorm_jobs(x_refs[1].at[NP // 2 - 1], h_refs[1], NP // 2 - 1)

    def attention_operand_jobs(p, slot, divide):
        inv = {}

        def sources(g, c):
            return {10 * h + b + 11: o_ref.at[2 * p + b, 4 * g + 2 * h + c] for h in range(2) for b in range(2)}

        def invert(g, c):
            def run(start):
                for k, src in sources(g, c).items():
                    inv[k] = 1.0 / _all8(jnp.add, _after(src[DH:], start))
                return token(*inv.values())
            return run

        def combine(g, c, r):
            def run(start):
                blocks = {k: src[_blk(r, 16)] * _tile(_after(inv[k], start), 2) if divide
                          else _after(src[_blk(r, 16)], start) for k, src in sources(g, c).items()}
                for i, terms in enumerate(RHS):
                    _put(op_refs[slot].at[z()], _blk(4 * g + 2 * c + r, 16), _blk(i), _combine(terms, blocks))
                return _fence(op_refs[slot])
            return run
        return [job for g in range(NG) for c in range(2)
                for job in [invert(g, c)] * divide + [combine(g, c, 0), combine(g, c, 1)]]

    def o_fence():
        return _bits(o_ref[0, H, :8])

    def input_jobs(p):
        moments, done = [_Moments(), _Moments()], []

        def transpose(c):
            def run(start):
                assert ("x", p) in arrived
                for b, mo in enumerate(moments):
                    x = io_ref[_blk(2 * p + b), _blk(c)]
                    x = (x if start is None else _bf16(_after(_bits(x), start))).T.astype(F32)
                    xa_refs[p % 2][p // 2, b, _blk(c)] = x
                    mo.add(x)
                return token(*[v for mo in moments for v in (mo.s1, mo.s2)])
            return run

        def stats():
            if not done:
                done.extend(mo.mean_and_scale() for mo in moments)
            return done
        return ([transpose(c) for c in range(NG)],
                normalize_jobs(xa_refs[p % 2].at[p // 2 + z()], h_refs[p % 2], p // 2, stats))

    def start_inputs(first, last):
        for p in range(first, min(last, NP)):
            x_copy(p).start()

    def prologue():
        start_inputs(0, 2)
        start_local_weights(0)
        z_ref[0] = 0
        zero_ref[...] = jnp.zeros((8, 128), U32)
        o_ref[0, H, :8] = jnp.zeros((8, 128), F32)
        for ref in (*tr_refs, wa_ref, wcur_ref, wb_ref, wo_ref, *h_refs, *op_refs):
            ref[(0,) * (len(ref.shape) - 2) + (slice(ref.shape[-2] - 8, None), _blk(0))] = jnp.zeros((8, 128), U32)
        (t0, n0), (t1, n1) = input_jobs(0), input_jobs(1)
        wait_input(0)
        start_inputs(2, 4)
        for job in t0:
            job(None)
        wait_input(1)
        for c, job in enumerate(t1):
            mark = job(None)
            for job in n0[2 * c:2 * c + 2]:
                job(mark)
        wait_local_weights(0)
        start_inputs(4, 6)
        jobs = qkv_weight_jobs(0, 0, wcur_ref)
        marks = [transpose(None) for transpose, _ in jobs[:3]]
        for n, (_, combine) in enumerate(jobs):
            marks += [transpose(None) for transpose, _ in jobs[n + 3:n + 4]]
            for job in combine:
                job(marks[n])
        return n1

    def local_jobs(g, staged, tag):
        weights, outs = {}, {}

        def load(refs, u, *index):
            assert staged[u // 2 % NS] == (tag, u // 2)
            return refs[u // 2 % NS][(u % 2 + z(), *index)]

        def window(u, a, c, start):
            lane = _after(lax.broadcasted_iota(jnp.int32, (8, 128), 1), start)
            cur = load(lkv_refs, u, _blk(a, DH // 2), _blk(c))
            if u:
                prev = load(lkv_refs, u - 1, _blk(a, DH // 2), _blk(c))
            else:
                prev = jnp.broadcast_to(cur[:, :1], cur.shape) if c else cur
            return lane, lambda w: _window_slot(cur, prev, w, lane)

        def weigh(u, a):
            def run(start):
                lane, k = window(u, a, 0, start)
                q = load(lq_refs, u, _blk(a, DH))
                t = _sum8([_tree(jnp.add, _rows8(q * k(w))) for w in range(WIN)])
                if u == 0:
                    t = jnp.where(lane >= DIL * lax.broadcasted_iota(jnp.int32, (8, 128), 0), t, MASKED)
                p = jnp.exp2(t - _all8(jnp.maximum, t))
                weights[u, a] = p / _all8(jnp.add, p)
                return token(weights[u, a])
            return run

        def gather(u, a):
            def run(start):
                _, v = window(u, a, 1, start)
                o = None
                for w in range(WIN):
                    t = v(w) * jnp.broadcast_to(weights[u, a][w:w + 1], (DH, 128))
                    o = t if o is None else o + t
                outs[u, a] = o
                return token(*_rows8(o))
            return run

        def store(u, a):
            def run(start):
                o_ref[u, 4 * g + a, :DH] = _after(outs[u, a], start)
                return o_fence()
            return run
        units = [(2 * p + b, a) for p in range(NP) for a in (2, 3, 0, 1) for b in range(2)]
        return [(weigh(*k), gather(*k), store(*k)) for k in units]

    slot_q = NB * MQ // 16
    span_q = NP * slot_q

    def qkv_local(rep, second_pair):
        def step(g):
            opening = isinstance(g, int)
            pacer = _Pacer(zero())
            staged = {} if opening else {p % NS: (-1, p) for p in range(NP)}
            units = [] if opening else local_jobs(jnp.maximum(g - 1, 0), staged, -1)[-LAG:]
            units += local_jobs(g, staged, 0)[:-LAG]
            w1, w2 = W_LOCAL[2 if opening else rep]
            first = 16 + (LAG * (span_q - 16) // (8 * NP) if opening else 0)
            pacer.spread([unit[0] for unit in units], first, span_q - 11, w1)
            pacer.spread([lambda start, unit=unit: (unit[1](start), unit[2](None))[1] for unit in units],
                         first + 10, span_q - 1, w2)
            nxt = (g + 1) % NG
            if opening:
                pacer.spread(second_pair, W_NORM, slot_q - 8, W_NORM)
                for p in range(2, NP):
                    transposes, normalize = input_jobs(p)
                    pacer.spread(transposes, (p - 2) * slot_q + W_XPOSE, (p - 1) * slot_q - 4, W_XPOSE)
                    pacer.spread(normalize, (p - 1) * slot_q + W_NORM - 8, p * slot_q - 8, W_NORM)
                pace_weights(pacer, out_weight_jobs(0, g), W_XPOSE, slot_q + W_XPOSE)
                pace_weights(pacer, qkv_weight_jobs(0, nxt), span_q - 2 * slot_q + W_XPOSE, span_q - 1)
            elif rep == 0:
                @pl.when(g + 1 < NG)
                def _():
                    wait_local_weights(g + 1)

                @pl.when(g + 2 < NG)
                def _():
                    start_local_weights(g + 2)

                @pl.when(g + 1 < NG)
                def _():
                    for piece in full_weight_copies(_blk(g + 1)):
                        piece.start()

                pace_weights(pacer, qkv_weight_jobs(0, nxt) + out_weight_jobs(0, g), W_XPOSE, span_q - 1)

                def copy(i, r):
                    def run(start):
                        wcur_ref[0, i, _blk(r, 24)] = _after(wa_ref[nxt + z(), i, _blk(r, 24)], start)
                        return _fence(wcur_ref, z())
                    return run
                pacer.spread([copy(i, r) for i in range(NB) for r in range(4)],
                             span_q - slot_q + W_COMBINE, span_q - 1, W_COMBINE)

            for p in range(NP):
                if opening and p % 2 == 0 and p + 2 < NP:
                    wait_input(p + 2)
                    wait_input(p + 3)
                    if p == 0:
                        start_inputs(6, NP)
                        start_local_weights(1)
                    if p == NP - 4:
                        wait_local_weights(1)
                        start_local_weights(2)
                        for piece in full_weight_copies(_blk(0, 256)):
                            piece.start()
                w_ref = wcur_ref.at[0] if opening or (rep == 0 and p < NP - 1) else wa_ref.at[g]
                r = pacer.block_product(lambda i: w_ref[i, :MQ // 2], h_operand(p, opening))
                staged[p % NS] = (0, p)
                for i, b in ((1, 0), (1, 1), (0, 0), (0, 1)):
                    kqv = r[10 * i + b + 11]
                    _put(lkv_refs[p % NS].at[b], _blk(i, 64), _blk(0), kqv[:64])
                    lq_refs[p % NS][b, _blk(i, 64)] = kqv[64:128] * QSCALE
                    _put(lkv_refs[p % NS].at[b], _blk(i, 64), _blk(1), kqv[128:])
            assert not pacer.jobs

        if rep == 0:
            step(0)
            wcur_ref[0, :, :MQ // 2] = wa_ref[1 + z(), :, :MQ // 2]
        else:
            for job in last_layernorm_jobs(xa_refs):
                job(None)
        pl.loop(1 - rep, NG)(step)

    def qkv_full(rep):
        @pl.loop(0, NG, step=GPB)
        def _(g0):
            pacer = _Pacer(zero())
            pacer.spread(last_layernorm_jobs(xb_refs), W_NORM, span_q - 2 * slot_q, W_NORM)
            for h in range(GPB):
                g = g0 + h
                if rep == 0:
                    first = h * span_q + 5 * MQ // 16
                    pace_weights(pacer, out_weight_jobs(1, g), first, first + span_q // 2 + W_COMBINE)
                for p in range(NP):
                    r = pacer.block_product(lambda i: wb_ref[g, i, :MQ // 2], h_operand(p, p == NP - 1))
                    for b in range(2):
                        u = 2 * p + b
                        k, q, v = [jnp.concatenate([r[11 + b][_blk(part, 64)], r[21 + b][_blk(part, 64)]], axis=0)
                                   for part in range(3)]
                        k_ref[g, _blk(u, 64), :] = _bits(k.astype(BF16).T)
                        _put(q_ref.at[g * NQ + u // 4], slice(None), _blk(u % 4), q * QSCALE)
                        _put(v_ref.at[g], slice(None), _blk(u), v)
            assert not pacer.jobs

    def values(item, a, c):
        return _bf16(v_ref[item // NQ, _blk(a, DH // 2), _blk(c, CK)])

    def store_head(item, a, acc, total):
        both = jnp.concatenate([acc, total], axis=0)
        for j in range(BQ // 128):
            o_ref[item % NQ * (BQ // 128) + j, item // NQ * 4 + a] = both[:, _blk(j)]

    def attend(item, first, last, jobs=()):
        tops, marks, due = {}, [], [[], []]
        top = total = acc = None
        for n in range(first, last):
            ahead, a = item + (n + SKEW) // 4, (n + SKEW) % 4
            q = _bf16(q_ref[ahead, _blk(a, DH // 2), :])
            q = jnp.concatenate([q if b == a else jnp.zeros_like(q) for b in range(4)], axis=0)
            if n >= 0:
                peak = tops[n % SKEW] if n % SKEW in tops else m_ref[n % SKEW]
            unreduced, total_before, acc_before = top, total, acc
            top = total = acc = None
            for c in range(NC):
                done = due.pop(0)
                due.append([])
                if c == 1 and unreduced is not None:
                    tops[(n - 1) % SKEW] = _all8(jnp.maximum, _after(unreduced, token(marks[0])))
                    due[-1].append(token(tops[(n - 1) % SKEW]))
                at, steps = (n - first) * NC + c, (last - first) * NC
                for job in jobs[at * len(jobs) // steps:(at + 1) * len(jobs) // steps]:
                    due[-1].append(job(token(marks[0][:, :128]) if marks else None))
                if n >= 0:
                    for t in done:
                        peak = _after(peak, t)
                    peaks = [_after(peak, token(mark)) for mark in marks[::2]] or [peak] * (CK // 32)
                    p, total = _exp_scores(lambda rows: s_refs[n % 4][c + z(), rows],
                                           [peaks[i // 2] for i in range(CK // 16)], total,
                                           None if total_before is None else token(total_before))
                s = _dot(_bf16(k_ref[ahead // NQ, _blk(c, CK // 2), :]), q)
                s_refs[a][c] = s
                link, marks = marks[-1:], []
                for i, slab in enumerate(_rows8(s)):
                    top = _after(slab, token(*link) if link else None) if top is None else jnp.maximum(top, slab)
                    if i % 2:
                        marks.append(top)
                if n >= 0:
                    o = _dot(values(item + n // 4, n % 4, c), p)
                    if acc is not None:
                        acc = acc + o
                    elif acc_before is not None:
                        acc = _after(o, _bits(acc_before) & _tile(zero(), DH // 8, BQ // 128))
                    else:
                        acc = o
            if n >= 0:
                store_head(item + n // 4, n % 4, acc, total)
        tops[(last - 1) % SKEW] = _all8(jnp.maximum, top)
        for slot, peak in tops.items():
            m_ref[slot] = peak

    def last_head_jobs(a):
        item, state = NG * NQ - 1, [None, None]

        def job(c):
            def run(start):
                p, state[0] = _exp_scores(lambda rows: s_refs[a][c + z(), rows],
                                          [_after(m_ref[a % SKEW + z()], start)] * (CK // 16), state[0], None)
                o = _dot(values(item, a, c), p)
                state[1] = o if state[1] is None else state[1] + o
                return token(*[x[:, _blk(j)] for x in (state[0], state[1][-8:]) for j in range(BQ // 128)])
            return run

        def store(start):
            store_head(item, a, _after(state[1], start), state[0])
            return start
        return [job(c) for c in range(NC)], store

    def attention():
        items = NG * NQ
        trips = (items - 1) // IPB
        lead = items - 1 - trips * IPB
        attend(0, -SKEW, 4 * lead)
        pl.loop(0, trips)(lambda i: attend(lead + i * IPB, 0, 4 * IPB))
        attend(items - 1, 0, 4 - SKEW, attention_operand_jobs(0, 0, True))

    span_o = NB * HD // 16

    def project(layer, t, src_refs, emit, add_jobs):
        pacer = _Pacer(zero())
        pacer.spread(attention_operand_jobs(2 * t + 1, 1, layer == 1), W_OPERAND, span_o - W_OPERAND, W_OPERAND)
        pacer.spread(attention_operand_jobs(jnp.minimum(2 * t + 2, NP - 1), 0, layer == 1),
                     span_o + W_OPERAND, 2 * span_o - 1, W_OPERAND)
        add_jobs(pacer)
        for pp in range(2):
            for j in range(HD // MO):
                r = pacer.block_product(lambda i: wo_ref[layer, i, _blk(j, MO // 2), :],
                                        lambda i: op_refs[pp][0, :HD // 2, _blk(i)])
                for c in range(MO // 64):
                    f = j * (MO // 64) + c
                    for b in range(2):
                        y = jnp.concatenate([r[11 + b][_blk(c, 64)], r[21 + b][_blk(c, 64)]], axis=0)
                        emit(pp, b, f, src_refs[pp][t, b, _blk(f)] + y)
        pacer.flush()
        assert not pacer.jobs

    def project_and_normalize(layer, t, src_refs, dst_refs, add_jobs):
        def emit(pp, b, f, x):
            dst_refs[pp][t, b, _blk(f)] = x

        def add_all(pacer):
            if not isinstance(t, int):
                pacer.spread(layernorm_jobs(dst_refs[1].at[t - 1], h_refs[1], t - 1), W_NORM, span_o - 1, W_NORM)
            pacer.spread(layernorm_jobs(dst_refs[0].at[t + z()], h_refs[0], t), span_o + W_NORM, 2 * span_o - 1, W_NORM)
            add_jobs(pacer)
        project(layer, t, src_refs, emit, add_all)

    def project_and_write(layer, t, src_refs, add_jobs):
        def emit(pp, b, f, x):
            io_ref[_blk(4 * t + 2 * pp + b), _blk(f)] = x.astype(BF16).T
            if b == 1 and f == NG - 1:
                out_copy(2 * t + pp).start()
        project(layer, t, src_refs, emit, add_jobs)

    def out_local(rep):
        def step(t):
            def add_jobs(pacer):
                if isinstance(t, int):
                    units = local_jobs(NG - 1, {p % NS: (0, p) for p in range(NP)}, 0)[-LAG:]
                    w1, w2 = W_LOCAL[0]
                    end = span_o + 16
                    pacer.spread([unit[0] for unit in units], w1, end - 10, w1)
                    pacer.spread([unit[1] for unit in units], w1 + 10, end, w2)
                    pacer.spread([unit[2] for unit in units], w1 + 10 + W_NORM, end + W_NORM, W_NORM)
                if rep == 0:
                    pace_weights(pacer, qkv_weight_jobs(1, 2 * t) + qkv_weight_jobs(1, 2 * t + 1),
                                 W_XPOSE, 2 * span_o - 1)
            project_and_normalize(0, t, xa_refs, xb_refs, add_jobs)
        for job in attention_operand_jobs(0, 0, False):
            job(None)
        step(0)
        pl.loop(1, NP // 2)(step)

    def out_full(rep):
        def finish_attention(pacer):
            tick = MO // 16
            heads = [last_head_jobs(a) for a in range(4 - SKEW, 4)]
            slots = 2 * span_o // tick
            for i, (chunks, store) in enumerate(heads):
                for c, job in enumerate(chunks):
                    start = (i * NC + c) * slots // (SKEW * NC) * tick
                    pacer.spread([job], start + W_VALUES, start + W_VALUES, W_VALUES)
                start = min(start + W_VALUES, 2 * span_o - 1)
                pacer.spread([store], start + tick, start + tick, tick)

        def step(t, add_jobs):
            if rep == 0:
                project_and_normalize(1, t, xb_refs, xa_refs, add_jobs)
            else:
                project_and_write(1, t, xb_refs, add_jobs)
        step(0, finish_attention)
        pl.loop(1, NP // 2)(lambda t: step(t, lambda pacer: None))

    second_pair = prologue()
    for rep in range(2):
        qkv_local(rep, second_pair)
        if rep == 0:
            for whole in full_weight_copies(slice(None)):
                whole.wait()
        out_local(rep)
        qkv_full(rep)
        attention()
        out_full(rep)
    for p in range(NP):
        out_copy(p).wait()


@jax.jit
def pallas_interleave_layers__sliding_local_dilated__softmax_full_mha__prompt_kernel(
    A_x: jax.Array,
    A_wqkv: jax.Array,
    A_wo: jax.Array,
    B_x: jax.Array,
    B_wqkv: jax.Array,
    B_wo: jax.Array,
):
    del B_x
    assert A_x.shape == (1, S, D)
    vmem = pltpu.VMEM
    out = pl.pallas_call(
        _kernel,
        out_shape=jax.ShapeDtypeStruct((S, D), BF16),
        in_specs=[pl.BlockSpec(memory_space=pl.ANY)] * 5,
        out_specs=pl.BlockSpec(memory_space=pl.ANY),
        scratch_shapes=[
            vmem((S, D), BF16),
            vmem((NG, 4, D, 128), BF16),
            vmem((D, 3 * D), BF16),
            vmem((D, D), BF16),
            [vmem((1, 2, 64 + 16, 128), U32)] * NTR,
            vmem((NG, NB, MQ // 2 + 8, HD), U32),
            vmem((1, NB, MQ // 2 + 8, HD), U32),
            vmem((NG, NB, MQ // 2 + 8, HD), U32),
            vmem((2, NB, HD // 2 + 8, HD), U32),
            [vmem((NP // 2, 2, D, 128), F32)] * 2,
            [vmem((NP // 2, 2, D, 128), F32)] * 2,
            [vmem((NP // 2, HD // 2 + 32, NB * 128), U32)] * 2,
            vmem((2 * NP, H + 4, DH + 8, 128), F32),
            [vmem((1, HD // 2 + 32, NB * 128), U32)] * 2,
            [vmem((2, 128, 128), F32)] * NS,
            [vmem((2, 64, 256), U32)] * NS,
            vmem((NG * NQ, 64, BQ), U32),
            vmem((NG, S // 2, 128), U32),
            vmem((NG, 64, S), U32),
            [vmem((NC, CK, BQ), F32)] * 4,
            vmem((SKEW, 8, BQ), F32),
            vmem((8, 128), U32),
            pltpu.SMEM((1,), jnp.int32),
            pltpu.SemaphoreType.DMA((NP,)),
            pltpu.SemaphoreType.DMA((NG,)),
            pltpu.SemaphoreType.DMA((2,)),
        ],
        compiler_params=pltpu.CompilerParams(vmem_limit_bytes=120 * 1024 * 1024),
        name="interleaved_attention_layers",
    )(A_x.reshape(S, D), A_wqkv, A_wo, B_wqkv, B_wo)
    return out.reshape(1, S, D)
```

```python
import math

import jax
import jax.numpy as jnp
from jax import lax
import jax.experimental.pallas as pl
import jax.experimental.pallas.tpu as pltpu

S = 2048
D = 1024
H = 32
DH = D // H
WIN, DIL = 8, 2
EPS = 1e-5
LOG2E = math.log2(math.e)
QSCALE = DH ** -0.5 * LOG2E
MASKED = -1e9 * LOG2E

HD = D // 2
NG = D // 128
NP = S // 256
MQ = 192
MO = 256
BQ = 512
NQ = S // BQ
CK = 128
NC = S // CK

NS = 2
LAG = 7
SKEW = 2
IPB = 2
GPB = 2

W_LOCAL = ((36, 30), (30, 24), (34, 28))
W_XPOSE, W_COPY, W_NORM, W_OPERAND, W_VALUES = 28, 14, 20, 20, 26

F32 = jnp.float32
BF16 = jnp.bfloat16
U32 = jnp.uint32


def _blk(i, n=128):
    return slice(i * n, (i + 1) * n) if isinstance(i, int) else pl.ds(pl.multiple_of(i * n, n), n)


def _dot(a, b):
    return jnp.dot(a, b, preferred_element_type=F32)


def _bits(x):
    return pltpu.bitcast(x, U32)


def _bf16(x):
    return pltpu.bitcast(x, BF16)


def _put(ref, rows, cols, x):
    ref.bitcast(BF16)[rows, cols] = x.astype(BF16)


def _rows8(x):
    return [x[r:r + 8] for r in range(0, x.shape[0], 8)]


def _tile(x, rows, cols=1):
    if cols > 1:
        x = jnp.concatenate([x] * cols, axis=1)
    return jnp.concatenate([x] * rows, axis=0) if rows > 1 else x


def _tree(op, xs):
    while len(xs) > 1:
        xs = [op(xs[i], xs[i + 1]) if i + 1 < len(xs) else xs[i] for i in range(0, len(xs), 2)]
    return xs[0]


def _all8(op, x):
    for sh in (4, 2, 1):
        x = op(x, pltpu.roll(x, sh, 0))
    return x


def _sum8(xs):
    row = lax.broadcasted_iota(jnp.int32, xs[0].shape, 0)
    low = (row & 4) == 0
    xs = [jnp.where(low, a, b) + pltpu.roll(jnp.where(low, b, a), 4, 0) for a, b in zip(xs[:4], xs[4:])]
    for sh in (2, 1):
        low = (row & sh) == 0
        xs = [jnp.where(low, a + pltpu.roll(a, 8 - sh, 0), b + pltpu.roll(b, sh, 0))
              for a, b in zip(xs[:sh], xs[sh:])]
    return xs[0]


def _after(x, token):
    if token is None:
        return x
    token = _tile(token, x.shape[0] // token.shape[0], x.shape[1] // token.shape[1])
    return pltpu.bitcast(_bits(x) | token, x.dtype)


def _fence(ref, z=0):
    return _bits(ref[(z,) + (0,) * (len(ref.shape) - 3) + (slice(ref.shape[-2] - 8, None), _blk(0))])


class _Pacer:
    def __init__(self, zero):
        self.zero = zero
        self.marks = []
        self.jobs = []
        self.due = {}

    def spread(self, jobs, first, last, window):
        for i, job in enumerate(jobs):
            due = first + (last - first) * i // max(len(jobs) - 1, 1)
            self.jobs.append((due - window, due, job))
        self.jobs.sort(key=lambda j: j[0])

    def flush(self):
        now = len(self.marks)
        while self.jobs and self.jobs[0][0] < now:
            start, due, job = self.jobs.pop(0)
            done = job(_bits(self.marks[start]) & self.zero if start >= 0 else None)
            self.due.setdefault(max(due, now), []).append(done)

    def product(self, lhs_ref, rows, rhs_ref, cols):
        out = None
        for h in range(D // HD):
            self.flush()
            now = len(self.marks)
            w = _rows8(lhs_ref[rows, _blk(h, HD)])
            for j, row in enumerate(w):
                if now + j in self.due:
                    w[j] = jnp.concatenate(
                        [row[:, :128] | _tree(jnp.bitwise_or, self.due[now + j]), row[:, 128:]], axis=1)
            m = _dot(_bf16(jnp.concatenate(w, axis=0)), _bf16(rhs_ref[_blk(h, HD // 2), cols]))
            self.marks += [m[16 * j:16 * j + 8] for j in range(len(w))]
            out = m if out is None else out + m
        return out


class _Moments:
    def __init__(self):
        self.x0 = self.s1 = self.s2 = None

    def add(self, x):
        for slab in _rows8(x):
            if self.x0 is None:
                self.x0 = slab
                continue
            d = slab - self.x0
            self.s1 = d if self.s1 is None else self.s1 + d
            self.s2 = d * d if self.s2 is None else self.s2 + d * d

    def mean_and_scale(self):
        n = D // 8
        mean = _all8(jnp.add, self.x0 + self.s1 * (1.0 / n)) * 0.125
        e = self.x0 - mean
        var = _all8(jnp.add, self.s2 + e * (2.0 * self.s1 + n * e)) * (1.0 / D)
        return mean, lax.rsqrt(jnp.maximum(var, 0.0) + EPS)


def _window_slot(cur, prev, w, lane):
    if w:
        cur = pltpu.roll(jnp.where(_tile(lane, 2) >= 128 - DIL * w, prev, cur), DIL * w, 1)
    return _bf16(cur).astype(F32)


def _exp_scores(scores, tops, total, link):
    p = []
    for i in range(CK // 16):
        e = jnp.exp2(scores(_blk(CK // 16 - 1 - i, 16)) - _tile(tops[i], 2))
        total = _after(e[:8] + e[8:], link) if total is None else total + (e[:8] + e[8:])
        p.append(e)
    return jnp.concatenate(p[::-1], axis=0).astype(BF16), total


def _kernel(x_hbm, aqkv_hbm, ao_hbm, bqkv_hbm, bo_hbm, out_hbm,
            io_ref, rawa_ref, rawb_ref, rawo_ref, wa_ref, wcur_ref, wb_ref, wo_ref,
            xa_refs, xb_refs, h_refs, lo_ref, o_ref, op_refs, lq_refs, lkv_refs,
            q_ref, k_ref, v_ref, s_refs, m_ref, zero_ref, z_ref, xsem, asem, bsem):

    def zero():
        return zero_ref[...]

    def z():
        return z_ref[0]

    def token(*values):
        return _tree(jnp.bitwise_or, [_bits(v) for v in values]) & _tile(zero(), 1, values[0].shape[1] // 128)

    arrived = set()

    def x_copy(p):
        return pltpu.make_async_copy(x_hbm.at[_blk(p, 256)], io_ref.at[_blk(p, 256)], xsem.at[p])

    def out_copy(p, cols):
        return pltpu.make_async_copy(io_ref.at[_blk(p, 256), cols], out_hbm.at[_blk(p, 256), cols], xsem.at[p])

    def start_local_weights(g):
        srcs = [aqkv_hbm.at[:, _blk(part * NG + g)] for part in range(3)] + [ao_hbm.at[:, _blk(g)]]
        for i, src in enumerate(srcs):
            pltpu.make_async_copy(src, rawa_ref.at[g, i], asem.at[g]).start()

    def wait_local_weights(g):
        pltpu.make_async_copy(rawa_ref.at[g], rawa_ref.at[g], asem.at[g]).wait()
        if isinstance(g, int):
            arrived.add(("w", g))

    def wait_input(p):
        x_copy(p).wait()
        arrived.add(("x", p))

    def full_weight_copies(rows):
        return [pltpu.make_async_copy(src.at[rows], dst.at[rows], bsem.at[i])
                for i, (src, dst) in enumerate(((bqkv_hbm, rawb_ref), (bo_hbm, rawo_ref)))]

    def weight_jobs(tile, dst_ref, index, rows):
        def job(c):
            def run(start):
                for r in (2 * c, 2 * c + 1):
                    t = tile(r) if start is None else _bf16(_after(_bits(tile(r)), start))
                    t = _bits(t.T)
                    for i, row in enumerate(rows):
                        dst_ref[index, _blk(row, 32), _blk(r)] = t[_blk(i, 32)]
                return _fence(dst_ref, z())
            return run
        return [job(c) for c in range(NG // 2)]

    def qkv_weight_jobs(layer, g, dst_ref):
        def tile(part, r):
            assert layer or not isinstance(g, int) or ("w", g) in arrived
            return rawb_ref[_blk(r), _blk(part * NG + g)] if layer else rawa_ref[g, part, _blk(r), :]
        return [job for row, part in enumerate((1, 0, 2))
                for job in weight_jobs(lambda r, part=part: tile(part, r), dst_ref, g, (row, row + 3))]

    def out_weight_jobs(layer, g):
        return weight_jobs(lambda r: rawo_ref[_blk(r), _blk(g)] if layer else rawa_ref[g, 3, _blk(r), :],
                           wo_ref, layer, (2 * g, 2 * g + 1))

    def normalized(p, fresh):
        return h_refs[p % 2].at[p // 2 + (z() if fresh else 0)]

    def normalize_jobs(x_ref, dst_ref, index, stats):
        def job(r):
            def run(start):
                for b, (mean, scale) in enumerate(stats()):
                    _put(dst_ref.at[index], _blk(r, 64), _blk(b),
                         (x_ref[b, _blk(r, 64)] - _tile(_after(mean, start), 8)) * _tile(scale, 8))
                return _fence(dst_ref, z())
            return run
        return [job(r) for r in range(D // 64)]

    def layernorm_jobs(x_ref, dst_ref, index):
        moments, done = [_Moments(), _Moments()], []

        def measure(c):
            def run(start):
                for b, mo in enumerate(moments):
                    if mo.x0 is not None:
                        mo.x0 = _after(mo.x0, start)
                    mo.add(x_ref[b, _blk(c)])
                return token(*[v for mo in moments for v in (mo.s1, mo.s2)])
            return run

        def stats():
            if not done:
                done.extend(mo.mean_and_scale() for mo in moments)
            return done
        return [measure(c) for c in range(NG)] + normalize_jobs(x_ref, dst_ref, index, stats)

    def last_layernorm_jobs(x_refs):
        return layernorm_jobs(x_refs[1].at[NP // 2 - 1], h_refs[1], NP // 2 - 1)

    def divide_jobs(p, slot):
        def job(head):
            def run(start):
                for b in range(2):
                    src = o_ref.at[2 * p + b, head]
                    inv = 1.0 / _all8(jnp.add, _after(src[DH:], start))
                    _put(op_refs[slot].at[z()], _blk(head, DH), _blk(b), src[:DH] * _tile(inv, DH // 8))
                return _fence(op_refs[slot])
            return run
        return [job(head) for head in range(H)]

    def input_jobs(p):
        moments, done = [_Moments(), _Moments()], []

        def transpose(c):
            def run(start):
                assert ("x", p) in arrived
                for b, mo in enumerate(moments):
                    x = io_ref[_blk(2 * p + b), _blk(c)]
                    x = (x if start is None else _bf16(_after(_bits(x), start))).T.astype(F32)
                    xa_refs[p % 2][p // 2, b, _blk(c)] = x
                    mo.add(x)
                return token(*[v for mo in moments for v in (mo.s1, mo.s2)])
            return run

        def stats():
            if not done:
                done.extend(mo.mean_and_scale() for mo in moments)
            return done
        return ([transpose(c) for c in range(NG)],
                normalize_jobs(xa_refs[p % 2].at[p // 2 + z()], h_refs[p % 2], p // 2, stats))

    def start_inputs(first, last):
        for p in range(first, min(last, NP)):
            x_copy(p).start()

    def prologue():
        start_inputs(0, 2)
        start_local_weights(0)
        z_ref[0] = 0
        zero_ref[...] = jnp.zeros((8, 128), U32)
        for ref in (wa_ref, wcur_ref, wb_ref, wo_ref, *h_refs, lo_ref, *op_refs):
            ref[(0,) * (len(ref.shape) - 2) + (slice(ref.shape[-2] - 8, None), _blk(0))] = jnp.zeros((8, 128), U32)
        (t0, n0), (t1, n1) = input_jobs(0), input_jobs(1)
        wait_input(0)
        start_inputs(2, 4)
        for job in t0:
            job(None)
        wait_input(1)
        for c, job in enumerate(t1):
            mark = job(None)
            for job in n0[2 * c:2 * c + 2]:
                job(mark)
        wait_local_weights(0)
        start_inputs(4, 6)
        for job in qkv_weight_jobs(0, 0, wcur_ref):
            job(None)
        return n1

    def local_jobs(g, staged, tag):
        weights = {}

        def load(refs, u, a, *index):
            assert staged[u % (2 * NS), a // 2] == (tag, u)
            return refs[u % (2 * NS)][(z(), *index)]

        def window(u, a, c, start):
            lane = _after(lax.broadcasted_iota(jnp.int32, (8, 128), 1), start)
            cur = load(lkv_refs, u, a, _blk(a, DH // 2), _blk(c))
            if u:
                prev = load(lkv_refs, u - 1, a, _blk(a, DH // 2), _blk(c))
            else:
                prev = jnp.broadcast_to(cur[:, :1], cur.shape) if c else cur
            return lane, lambda w: _window_slot(cur, prev, w, lane)

        def weigh(u, a):
            def run(start):
                lane, k = window(u, a, 0, start)
                q = load(lq_refs, u, a, _blk(a, DH))
                t = _sum8([_tree(jnp.add, _rows8(q * k(w))) for w in range(WIN)])
                if u == 0:
                    t = jnp.where(lane >= DIL * lax.broadcasted_iota(jnp.int32, (8, 128), 0), t, MASKED)
                p = jnp.exp2(t - _all8(jnp.maximum, t))
                weights[u, a] = p / _all8(jnp.add, p)
                return token(weights[u, a])
            return run

        def gather(u, a):
            def run(start):
                _, v = window(u, a, 1, start)
                o = None
                for w in range(WIN):
                    t = v(w) * jnp.broadcast_to(weights[u, a][w:w + 1], (DH, 128))
                    o = t if o is None else o + t
                _put(lo_ref.at[u // 2], _blk(4 * g + a, DH), _blk(u % 2), o)
                return _fence(lo_ref, z())
            return run
        return [(weigh(u, a), gather(u, a)) for u in range(2 * NP) for a in range(4)]

    def staged_at_end(tag):
        return {(u % (2 * NS), i): (tag, u) for u in range(2 * NP) for i in range(2)}

    slot_q = 8 * MQ // 16
    span_q = NP * slot_q

    def qkv_local(rep, second_pair):
        def step(g):
            opening = isinstance(g, int)
            pacer = _Pacer(zero())
            staged = {} if opening else staged_at_end(-1)
            units = [] if opening else local_jobs(jnp.maximum(g - 1, 0), staged, -1)[-LAG:]
            units += local_jobs(g, staged, 0)[:-LAG]
            w1, w2 = W_LOCAL[2 if opening else rep]
            first = 16 + (LAG * (span_q - 16) // (8 * NP) if opening else 0)
            pacer.spread([unit[0] for unit in units], first, span_q - 11, w1)
            pacer.spread([unit[1] for unit in units], first + 10, span_q - 1, w2)
            nxt = (g + 1) % NG
            if opening:
                pacer.spread(second_pair, W_NORM, slot_q - 8, W_NORM)
                for p in range(2, NP):
                    transposes, normalize = input_jobs(p)
                    pacer.spread(transposes, (p - 2) * slot_q + W_XPOSE, (p - 1) * slot_q - 4, W_XPOSE)
                    pacer.spread(normalize, (p - 1) * slot_q + W_NORM - 8, p * slot_q - 8, W_NORM)
                pacer.spread(out_weight_jobs(0, g), W_XPOSE, slot_q, W_XPOSE)
                pacer.spread(qkv_weight_jobs(0, nxt, wa_ref), span_q - 2 * slot_q + W_XPOSE, span_q - 1, W_XPOSE)
            elif rep == 0:
                @pl.when(g + 1 < NG)
                def _():
                    wait_local_weights(g + 1)

                @pl.when(g + 2 < NG)
                def _():
                    start_local_weights(g + 2)

                @pl.when(g + 1 < NG)
                def _():
                    for piece in full_weight_copies(_blk(g + 1)):
                        piece.start()

                pacer.spread(qkv_weight_jobs(0, nxt, wa_ref) + out_weight_jobs(0, g), W_XPOSE, span_q - 1, W_XPOSE)

                def copy(r):
                    def run(start):
                        wcur_ref[0, _blk(r, 8)] = _after(wa_ref[nxt + z(), _blk(r, 8)], start)
                        return _fence(wcur_ref, z())
                    return run
                pacer.spread([copy(r) for r in range(MQ // 8)], span_q - slot_q + W_COPY, span_q - 1, W_COPY)

            for p in range(NP):
                if opening and p % 2 == 0 and p + 2 < NP:
                    wait_input(p + 2)
                    wait_input(p + 3)
                    if p == 0:
                        start_inputs(6, NP)
                        start_local_weights(1)
                    if p == NP - 4:
                        wait_local_weights(1)
                        start_local_weights(2)
                        for piece in full_weight_copies(_blk(0, 256)):
                            piece.start()
                w_ref = wcur_ref.at[0] if opening or (rep == 0 and p < NP - 1) else wa_ref.at[g]
                for u in (2 * p, 2 * p + 1):
                    for i in range(2):
                        kqv = pacer.product(w_ref, _blk(i, MQ // 2), normalized(p, opening), _blk(u % 2))
                        staged[u % (2 * NS), i] = (0, u)
                        _put(lkv_refs[u % (2 * NS)].at[0], _blk(i, 64), _blk(0), kqv[:64])
                        lq_refs[u % (2 * NS)][0, _blk(i, 64)] = kqv[64:128] * QSCALE
                        _put(lkv_refs[u % (2 * NS)].at[0], _blk(i, 64), _blk(1), kqv[128:])
            assert not pacer.jobs

        if rep == 0:
            step(0)
            wcur_ref[0, :MQ] = wa_ref[1 + z(), :MQ]
        else:
            for job in last_layernorm_jobs(xa_refs):
                job(None)
        pl.loop(1 - rep, NG)(step)

    def qkv_full(rep):
        @pl.loop(0, NG, step=GPB)
        def _(g0):
            pacer = _Pacer(zero())
            pacer.spread(last_layernorm_jobs(xb_refs), W_NORM, span_q - 2 * slot_q, W_NORM)
            for h in range(GPB):
                g = g0 + h
                if rep == 0:
                    first = h * span_q + slot_q // 2
                    pacer.spread(out_weight_jobs(1, g), first, first + 3 * slot_q, W_XPOSE)
                for u in range(2 * NP):
                    kqv = [pacer.product(wb_ref.at[g], _blk(i, MQ // 2), normalized(u // 2, u // 2 == NP - 1),
                                         _blk(u % 2)) for i in range(2)]
                    for i in range(2):
                        _put(q_ref.at[g * NQ + u // 4], _blk(i, 64), _blk(u % 4), kqv[i][64:128] * QSCALE)
                        _put(v_ref.at[g], _blk(i, 64), _blk(u), kqv[i][128:])
                    k_ref[g, _blk(u, 64), :] = _bits(jnp.concatenate([x[:64] for x in kqv], axis=0).astype(BF16).T)
            assert not pacer.jobs

    def values(item, a, c):
        return _bf16(v_ref[item // NQ, _blk(a, DH // 2), _blk(c, CK)])

    def store_head(item, a, acc, total):
        both = jnp.concatenate([acc, total], axis=0)
        for j in range(BQ // 128):
            o_ref[item % NQ * (BQ // 128) + j, item // NQ * 4 + a] = both[:, _blk(j)]

    def attend(item, first, last, jobs=()):
        tops, marks, due = {}, [], [[], []]
        top = total = acc = None
        for n in range(first, last):
            ahead, a = item + (n + SKEW) // 4, (n + SKEW) % 4
            q = _bf16(q_ref[ahead, _blk(a, DH // 2), :])
            q = jnp.concatenate([q if b == a else jnp.zeros_like(q) for b in range(4)], axis=0)
            if n >= 0:
                peak = tops[n % SKEW] if n % SKEW in tops else m_ref[n % SKEW]
            unreduced, total_before, acc_before = top, total, acc
            top = total = acc = None
            for c in range(NC):
                done = due.pop(0)
                due.append([])
                if c == 1 and unreduced is not None:
                    tops[(n - 1) % SKEW] = _all8(jnp.maximum, _after(unreduced, token(marks[0])))
                    due[-1].append(token(tops[(n - 1) % SKEW]))
                at, steps = (n - first) * NC + c, (last - first) * NC
                for job in jobs[at * len(jobs) // steps:(at + 1) * len(jobs) // steps]:
                    due[-1].append(job(token(marks[0][:, :128]) if marks else None))
                if n >= 0:
                    for t in done:
                        peak = _after(peak, t)
                    peaks = [_after(peak, token(mark)) for mark in marks[::2]] or [peak] * (CK // 32)
                    p, total = _exp_scores(lambda rows: s_refs[n % 4][c + z(), rows],
                                           [peaks[i // 2] for i in range(CK // 16)], total,
                                           None if total_before is None else token(total_before))
                s = _dot(_bf16(k_ref[ahead // NQ, _blk(c, CK // 2), :]), q)
                s_refs[a][c] = s
                link, marks = marks[-1:], []
                for i, slab in enumerate(_rows8(s)):
                    top = _after(slab, token(*link) if link else None) if top is None else jnp.maximum(top, slab)
                    if i % 2:
                        marks.append(top)
                if n >= 0:
                    o = _dot(values(item + n // 4, n % 4, c), p)
                    if acc is not None:
                        acc = acc + o
                    elif acc_before is not None:
                        acc = _after(o, _bits(acc_before) & _tile(zero(), DH // 8, BQ // 128))
                    else:
                        acc = o
            if n >= 0:
                store_head(item + n // 4, n % 4, acc, total)
        tops[(last - 1) % SKEW] = _all8(jnp.maximum, top)
        for slot, peak in tops.items():
            m_ref[slot] = peak

    def last_head_jobs(a):
        item, state = NG * NQ - 1, [None, None]

        def job(c):
            def run(start):
                p, state[0] = _exp_scores(lambda rows: s_refs[a][c + z(), rows],
                                          [_after(m_ref[a % SKEW + z()], start)] * (CK // 16), state[0], None)
                o = _dot(values(item, a, c), p)
                state[1] = o if state[1] is None else state[1] + o
                return token(*[x[:, _blk(j)] for x in (state[0], state[1][-8:]) for j in range(BQ // 128)])
            return run

        def store(start):
            store_head(item, a, _after(state[1], start), state[0])
            return start
        return [job(c) for c in range(NC)], store

    def attention():
        items = NG * NQ
        trips = (items - 1) // IPB
        lead = items - 1 - trips * IPB
        attend(0, -SKEW, 4 * lead)
        pl.loop(0, trips)(lambda i: attend(lead + i * IPB, 0, 4 * IPB))
        attend(items - 1, 0, 4 - SKEW, divide_jobs(0, 0))

    span_o = 4 * D // 16

    def project(layer, t, src_refs, emit, add_jobs):
        pacer = _Pacer(zero())
        if layer:
            pacer.spread(divide_jobs(2 * t + 1, 1), W_OPERAND, span_o - W_OPERAND, W_OPERAND)
            pacer.spread(divide_jobs(jnp.minimum(2 * t + 2, NP - 1), 0), span_o + W_OPERAND, 2 * span_o - 1, W_OPERAND)
        add_jobs(pacer)
        for pp in range(2):
            attended = op_refs[pp].at[0] if layer else lo_ref.at[2 * t + pp]
            for j in range(D // MO):
                for b in range(2):
                    y = pacer.product(wo_ref.at[layer], _blk(j, MO // 2), attended, _blk(b))
                    for c in range(MO // 128):
                        f = j * (MO // 128) + c
                        emit(pp, b, f, src_refs[pp][t, b, _blk(f)] + y[_blk(c)])
        pacer.flush()
        assert not pacer.jobs

    def project_and_normalize(layer, t, src_refs, dst_refs, add_jobs):
        def emit(pp, b, f, x):
            dst_refs[pp][t, b, _blk(f)] = x

        def add_all(pacer):
            if not isinstance(t, int):
                pacer.spread(layernorm_jobs(dst_refs[1].at[t - 1], h_refs[1], t - 1), W_NORM, span_o - 1, W_NORM)
            pacer.spread(layernorm_jobs(dst_refs[0].at[t + z()], h_refs[0], t), span_o + W_NORM, 2 * span_o - 1, W_NORM)
            add_jobs(pacer)
        project(layer, t, src_refs, emit, add_all)

    def project_and_write(layer, t, src_refs, add_jobs):
        def emit(pp, b, f, x):
            io_ref[_blk(4 * t + 2 * pp + b), _blk(f)] = x.astype(BF16).T
            if b == 1 and (f + 1) % (NG // 2) == 0:
                out_copy(2 * t + pp, _blk(f // (NG // 2), HD)).start()
        project(layer, t, src_refs, emit, add_jobs)

    def out_local(rep):
        def step(t):
            def add_jobs(pacer):
                if isinstance(t, int):
                    units = local_jobs(NG - 1, staged_at_end(0), 0)[-LAG:]
                    w1, w2 = W_LOCAL[0]
                    end = span_o + 16
                    pacer.spread([unit[0] for unit in units], w1, end - 10, w1)
                    pacer.spread([unit[1] for unit in units], w1 + 10, end, w2)
                if rep == 0:
                    pacer.spread(qkv_weight_jobs(1, 2 * t, wb_ref) + qkv_weight_jobs(1, 2 * t + 1, wb_ref),
                                 W_XPOSE, 2 * span_o - 1, W_XPOSE)
            project_and_normalize(0, t, xa_refs, xb_refs, add_jobs)
        step(0)
        pl.loop(1, NP // 2)(step)

    def out_full(rep):
        def finish_attention(pacer):
            tick = MO // 16
            heads = [last_head_jobs(a) for a in range(4 - SKEW, 4)]
            slots = 2 * span_o // tick
            for i, (chunks, store) in enumerate(heads):
                for c, job in enumerate(chunks):
                    start = (i * NC + c) * slots // (SKEW * NC) * tick
                    pacer.spread([job], start + W_VALUES, start + W_VALUES, W_VALUES)
                start = min(start + W_VALUES, 2 * span_o - 1)
                pacer.spread([store], start + tick, start + tick, tick)

        def step(t, add_jobs):
            if rep == 0:
                project_and_normalize(1, t, xb_refs, xa_refs, add_jobs)
            else:
                project_and_write(1, t, xb_refs, add_jobs)
        step(0, finish_attention)
        pl.loop(1, NP // 2)(lambda t: step(t, lambda pacer: None))

    second_pair = prologue()
    for rep in range(2):
        qkv_local(rep, second_pair)
        if rep == 0:
            for whole in full_weight_copies(slice(None)):
                whole.wait()
        out_local(rep)
        qkv_full(rep)
        attention()
        out_full(rep)
    for p in range(NP):
        out_copy(p, slice(None)).wait()


@jax.jit
def pallas_interleave_layers__sliding_local_dilated__softmax_full_mha__prompt_kernel(
    A_x: jax.Array,
    A_wqkv: jax.Array,
    A_wo: jax.Array,
    B_x: jax.Array,
    B_wqkv: jax.Array,
    B_wo: jax.Array,
):
    del B_x
    assert A_x.shape == (1, S, D)
    vmem = pltpu.VMEM
    out = pl.pallas_call(
        _kernel,
        out_shape=jax.ShapeDtypeStruct((S, D), BF16),
        in_specs=[pl.BlockSpec(memory_space=pl.ANY)] * 5,
        out_specs=pl.BlockSpec(memory_space=pl.ANY),
        scratch_shapes=[
            vmem((S, D), BF16),
            vmem((NG, 4, D, 128), BF16),
            vmem((D, 3 * D), BF16),
            vmem((D, D), BF16),
            vmem((NG, MQ + 8, D), U32),
            vmem((1, MQ + 8, D), U32),
            vmem((NG, MQ + 8, D), U32),
            vmem((2, D // 2 + 8, D), U32),
            [vmem((NP // 2, 2, D, 128), F32)] * 2,
            [vmem((NP // 2, 2, D, 128), F32)] * 2,
            [vmem((NP // 2, D // 2 + 16, 256), U32)] * 2,
            vmem((NP, D // 2 + 16, 256), U32),
            vmem((2 * NP, H, DH + 8, 128), F32),
            [vmem((1, D // 2 + 16, 256), U32)] * 2,
            [vmem((1, 128, 128), F32)] * (2 * NS),
            [vmem((1, 64, 256), U32)] * (2 * NS),
            vmem((NG * NQ, 64, BQ), U32),
            vmem((NG, S // 2, 128), U32),
            vmem((NG, 64, S), U32),
            [vmem((NC, CK, BQ), F32)] * 4,
            vmem((SKEW, 8, BQ), F32),
            vmem((8, 128), U32),
            pltpu.SMEM((1,), jnp.int32),
            pltpu.SemaphoreType.DMA((NP,)),
            pltpu.SemaphoreType.DMA((NG,)),
            pltpu.SemaphoreType.DMA((2,)),
        ],
        compiler_params=pltpu.CompilerParams(vmem_limit_bytes=112 * 1024 * 1024),
        name="interleaved_attention_layers",
    )(A_x.reshape(S, D), A_wqkv, A_wo, B_wqkv, B_wo)
    return out.reshape(1, S, D)
```

```python
import math

import jax
import jax.numpy as jnp
from jax import lax
import jax.experimental.pallas as pl
import jax.experimental.pallas.tpu as pltpu

S = 2048
D = 1024
H = 32
DH = D // H
WIN, DIL = 8, 2
EPS = 1e-5
LOG2E = math.log2(math.e)
QSCALE = DH ** -0.5 * LOG2E
MASKED = -1e9 * LOG2E

HD = D // 2
NG = D // 128
NP = S // 256
MQ = 192
MO = 256
BQ = 512
NQ = S // BQ
CK = 128
NC = S // CK

NS = 2
LAG = 8
SKEW = 2
IPB = 2
GPB = 2

W_LOCAL = ((38, 32), (34, 28), (38, 32))
W_XPOSE, W_COPY, W_NORM, W_OPERAND, W_VALUES = 38, 14, 20, 20, 26

F32 = jnp.float32
BF16 = jnp.bfloat16
U32 = jnp.uint32


def _blk(i, n=128):
    return slice(i * n, (i + 1) * n) if isinstance(i, int) else pl.ds(pl.multiple_of(i * n, n), n)


def _dot(a, b):
    return jnp.dot(a, b, preferred_element_type=F32)


def _bits(x):
    return pltpu.bitcast(x, U32)


def _bf16(x):
    return pltpu.bitcast(x, BF16)


def _put(ref, rows, cols, x):
    ref.bitcast(BF16)[rows, cols] = x.astype(BF16)


def _rows8(x):
    return [x[r:r + 8] for r in range(0, x.shape[0], 8)]


def _tile(x, rows, cols=1):
    if cols > 1:
        x = jnp.concatenate([x] * cols, axis=1)
    return jnp.concatenate([x] * rows, axis=0) if rows > 1 else x


def _tree(op, xs):
    while len(xs) > 1:
        xs = [op(xs[i], xs[i + 1]) if i + 1 < len(xs) else xs[i] for i in range(0, len(xs), 2)]
    return xs[0]


def _all8(op, x):
    for sh in (4, 2, 1):
        x = op(x, pltpu.roll(x, sh, 0))
    return x


def _sum8(xs):
    row = lax.broadcasted_iota(jnp.int32, xs[0].shape, 0)
    low = (row & 4) == 0
    xs = [jnp.where(low, a, b) + pltpu.roll(jnp.where(low, b, a), 4, 0) for a, b in zip(xs[:4], xs[4:])]
    for sh in (2, 1):
        low = (row & sh) == 0
        xs = [jnp.where(low, a + pltpu.roll(a, 8 - sh, 0), b + pltpu.roll(b, sh, 0))
              for a, b in zip(xs[:sh], xs[sh:])]
    return xs[0]


def _after(x, token):
    if token is None:
        return x
    token = _tile(token, x.shape[0] // token.shape[0], x.shape[1] // token.shape[1])
    return pltpu.bitcast(_bits(x) | token, x.dtype)


def _fence(ref, z=0):
    return _bits(ref[(z,) + (0,) * (len(ref.shape) - 3) + (slice(ref.shape[-2] - 8, None), _blk(0))])


class _Pacer:
    def __init__(self, zero):
        self.zero = zero
        self.marks = []
        self.jobs = []
        self.due = {}

    def spread(self, jobs, first, last, window):
        for i, job in enumerate(jobs):
            due = first + (last - first) * i // max(len(jobs) - 1, 1)
            self.jobs.append((due - window, due, job))
        self.jobs.sort(key=lambda j: j[0])

    def flush(self):
        now = len(self.marks)
        while self.jobs and self.jobs[0][0] < now:
            start, due, job = self.jobs.pop(0)
            done = job(_bits(self.marks[start]) & self.zero if start >= 0 else None)
            self.due.setdefault(max(due, now), []).append(done)

    def product(self, lhs_ref, rows, rhs_ref, cols):
        out = None
        for h in range(D // HD):
            self.flush()
            now = len(self.marks)
            w = _rows8(lhs_ref[rows, _blk(h, HD)])
            for j, row in enumerate(w):
                if now + j in self.due:
                    w[j] = jnp.concatenate(
                        [row[:, :128] | _tree(jnp.bitwise_or, self.due[now + j]), row[:, 128:]], axis=1)
            m = _dot(_bf16(jnp.concatenate(w, axis=0)), _bf16(rhs_ref[_blk(h, HD // 2), cols]))
            self.marks += [m[16 * j:16 * j + 8] for j in range(len(w))]
            out = m if out is None else out + m
        return out


class _Moments:
    def __init__(self):
        self.x0 = self.s1 = self.s2 = None

    def add(self, x):
        for slab in _rows8(x):
            if self.x0 is None:
                self.x0 = slab
                continue
            d = slab - self.x0
            self.s1 = d if self.s1 is None else self.s1 + d
            self.s2 = d * d if self.s2 is None else self.s2 + d * d

    def mean_and_scale(self):
        n = D // 8
        mean = _all8(jnp.add, self.x0 + self.s1 * (1.0 / n)) * 0.125
        e = self.x0 - mean
        var = _all8(jnp.add, self.s2 + e * (2.0 * self.s1 + n * e)) * (1.0 / D)
        return mean, lax.rsqrt(jnp.maximum(var, 0.0) + EPS)


def _window_slot(cur, prev, w, lane):
    if w:
        cur = pltpu.roll(jnp.where(_tile(lane, 2) >= 128 - DIL * w, prev, cur), DIL * w, 1)
    return _bf16(cur).astype(F32)


def _exp_scores(scores, tops, total, link):
    p = []
    for i in range(CK // 16):
        e = jnp.exp2(scores(_blk(CK // 16 - 1 - i, 16)) - _tile(tops[i], 2))
        total = _after(e[:8] + e[8:], link) if total is None else total + (e[:8] + e[8:])
        p.append(e)
    return jnp.concatenate(p[::-1], axis=0).astype(BF16), total


def _kernel(x_hbm, aqkv_hbm, ao_hbm, bqkv_hbm, bo_hbm, out_hbm,
            io_ref, rawa_ref, rawb_ref, rawo_ref, wa_ref, wcur_ref, wb_ref, wo_ref,
            xa_refs, xb_refs, h_refs, lo_ref, o_ref, op_refs, lq_refs, lkv_refs,
            q_ref, k_ref, v_ref, s_refs, m_ref, zero_ref, z_ref, xsem, asem, bsem):

    def zero():
        return zero_ref[...]

    def z():
        return z_ref[0]

    def token(*values):
        return _tree(jnp.bitwise_or, [_bits(v) for v in values]) & _tile(zero(), 1, values[0].shape[1] // 128)

    arrived = set()

    def x_copy(p):
        return pltpu.make_async_copy(x_hbm.at[_blk(p, 256)], io_ref.at[_blk(p, 256)], xsem.at[p])

    def out_copy(p, cols):
        return pltpu.make_async_copy(io_ref.at[_blk(p, 256), cols], out_hbm.at[_blk(p, 256), cols], xsem.at[p])

    def start_local_weights(g):
        srcs = [aqkv_hbm.at[:, _blk(part * NG + g)] for part in range(3)] + [ao_hbm.at[:, _blk(g)]]
        for i, src in enumerate(srcs):
            pltpu.make_async_copy(src, rawa_ref.at[g, i], asem.at[g]).start()

    def wait_local_weights(g):
        pltpu.make_async_copy(rawa_ref.at[g], rawa_ref.at[g], asem.at[g]).wait()
        if isinstance(g, int):
            arrived.add(("w", g))

    def wait_input(p):
        x_copy(p).wait()
        arrived.add(("x", p))

    def full_weight_copies(rows):
        return [pltpu.make_async_copy(src.at[rows], dst.at[rows], bsem.at[i])
                for i, (src, dst) in enumerate(((bqkv_hbm, rawb_ref), (bo_hbm, rawo_ref)))]

    def weight_jobs(tile, dst_ref, index, rows):
        def job(c):
            def run(start):
                for r in (2 * c, 2 * c + 1):
                    t = tile(r) if start is None else _bf16(_after(_bits(tile(r)), start))
                    t = _bits(t.T)
                    for i, row in enumerate(rows):
                        dst_ref[index, _blk(row, 32), _blk(r)] = t[_blk(i, 32)]
                return _fence(dst_ref, z())
            return run
        return [job(c) for c in range(NG // 2)]

    def qkv_weight_jobs(layer, g, dst_ref):
        def tile(part, r):
            assert layer or not isinstance(g, int) or ("w", g) in arrived
            return rawb_ref[_blk(r), _blk(part * NG + g)] if layer else rawa_ref[g, part, _blk(r), :]
        return [job for row, part in enumerate((1, 0, 2))
                for job in weight_jobs(lambda r, part=part: tile(part, r), dst_ref, g, (row, row + 3))]

    def out_weight_jobs(layer, g):
        return weight_jobs(lambda r: rawo_ref[_blk(r), _blk(g)] if layer else rawa_ref[g, 3, _blk(r), :],
                           wo_ref, layer, (2 * g, 2 * g + 1))

    def normalized(p, fresh):
        return h_refs[p % 2].at[p // 2 + (z() if fresh else 0)]

    def normalize_jobs(x_ref, dst_ref, index, stats):
        def job(r):
            def run(start):
                for b, (mean, scale) in enumerate(stats()):
                    _put(dst_ref.at[index], _blk(r, 64), _blk(b),
                         (x_ref[b, _blk(r, 64)] - _tile(_after(mean, start), 8)) * _tile(scale, 8))
                return _fence(dst_ref, z())
            return run
        return [job(r) for r in range(D // 64)]

    def layernorm_jobs(x_ref, dst_ref, index):
        moments, done = [_Moments(), _Moments()], []

        def measure(c):
            def run(start):
                for b, mo in enumerate(moments):
                    if mo.x0 is not None:
                        mo.x0 = _after(mo.x0, start)
                    mo.add(x_ref[b, _blk(c)])
                return token(*[v for mo in moments for v in (mo.s1, mo.s2)])
            return run

        def stats():
            if not done:
                done.extend(mo.mean_and_scale() for mo in moments)
            return done
        return [measure(c) for c in range(NG)] + normalize_jobs(x_ref, dst_ref, index, stats)

    def last_layernorm_jobs(x_refs):
        return layernorm_jobs(x_refs[1].at[NP // 2 - 1], h_refs[1], NP // 2 - 1)

    def divide_jobs(p, slot):
        def job(head):
            def run(start):
                for b in range(2):
                    src = o_ref.at[2 * p + b, head]
                    inv = 1.0 / _all8(jnp.add, _after(src[DH:], start))
                    _put(op_refs[slot].at[z()], _blk(head, DH), _blk(b), src[:DH] * _tile(inv, DH // 8))
                return _fence(op_refs[slot])
            return run
        return [job(head) for head in range(H)]

    def input_jobs(p):
        moments, done = [_Moments(), _Moments()], []

        def transpose(c):
            def run(start):
                assert ("x", p) in arrived
                for b, mo in enumerate(moments):
                    x = io_ref[_blk(2 * p + b), _blk(c)]
                    x = (x if start is None else _bf16(_after(_bits(x), start))).T.astype(F32)
                    xa_refs[p % 2][p // 2, b, _blk(c)] = x
                    mo.add(x)
                return token(*[v for mo in moments for v in (mo.s1, mo.s2)])
            return run

        def stats():
            if not done:
                done.extend(mo.mean_and_scale() for mo in moments)
            return done
        return ([transpose(c) for c in range(NG)],
                normalize_jobs(xa_refs[p % 2].at[p // 2 + z()], h_refs[p % 2], p // 2, stats))

    def start_inputs(first, last):
        for p in range(first, min(last, NP)):
            x_copy(p).start()

    def prologue():
        start_inputs(0, 2)
        start_local_weights(0)
        z_ref[0] = 0
        zero_ref[...] = jnp.zeros((8, 128), U32)
        for ref in (wa_ref, wcur_ref, wb_ref, wo_ref, *h_refs, lo_ref, *op_refs):
            ref[(0,) * (len(ref.shape) - 2) + (slice(ref.shape[-2] - 8, None), _blk(0))] = jnp.zeros((8, 128), U32)
        (t0, n0), (t1, n1) = input_jobs(0), input_jobs(1)
        wait_input(0)
        start_inputs(2, 4)
        for job in t0:
            job(None)
        wait_input(1)
        for c, job in enumerate(t1):
            mark = job(None)
            for job in n0[2 * c:2 * c + 2]:
                job(mark)
        wait_local_weights(0)
        start_inputs(4, 6)
        for job in qkv_weight_jobs(0, 0, wcur_ref):
            job(None)
        return n1

    def local_jobs(g, staged, tag):
        weights = {}

        def load(refs, u, a, *index):
            assert staged[u % (2 * NS), a // 2] == (tag, u)
            return refs[u % (2 * NS)][(z(), *index)]

        def window(u, a, c, start):
            lane = _after(lax.broadcasted_iota(jnp.int32, (8, 128), 1), start)
            cur = load(lkv_refs, u, a, _blk(a, DH // 2), _blk(c))
            if u:
                prev = load(lkv_refs, u - 1, a, _blk(a, DH // 2), _blk(c))
            else:
                prev = jnp.broadcast_to(cur[:, :1], cur.shape) if c else cur
            return lane, lambda w: _window_slot(cur, prev, w, lane)

        def weigh(u, a):
            def run(start):
                lane, k = window(u, a, 0, start)
                q = load(lq_refs, u, a, _blk(a, DH))
                t = _sum8([_tree(jnp.add, _rows8(q * k(w))) for w in range(WIN)])
                if u == 0:
                    t = jnp.where(lane >= DIL * lax.broadcasted_iota(jnp.int32, (8, 128), 0), t, MASKED)
                p = jnp.exp2(t - _all8(jnp.maximum, t))
                weights[u, a] = p / _all8(jnp.add, p)
                return token(weights[u, a])
            return run

        def gather(u, a):
            def run(start):
                _, v = window(u, a, 1, start)
                o = None
                for w in range(WIN):
                    t = v(w) * jnp.broadcast_to(weights[u, a][w:w + 1], (DH, 128))
                    o = t if o is None else o + t
                _put(lo_ref.at[u // 2], _blk(4 * g + a, DH), _blk(u % 2), o)
                return _fence(lo_ref, z())
            return run
        return [(weigh(u, a), gather(u, a)) for u in range(2 * NP) for a in range(4)]

    def staged_at_end(tag):
        return {(u % (2 * NS), i): (tag, u) for u in range(2 * NP) for i in range(2)}

    slot_q = 8 * MQ // 16
    span_q = NP * slot_q

    def qkv_local(rep, second_pair):
        def step(g):
            opening = isinstance(g, int)
            pacer = _Pacer(zero())
            staged = {} if opening else staged_at_end(-1)
            units = [] if opening else local_jobs(jnp.maximum(g - 1, 0), staged, -1)[-LAG:]
            units += local_jobs(g, staged, 0)[:-LAG]
            w1, w2 = W_LOCAL[2 if opening else rep]
            first = 26 + (LAG * (span_q - 16) // (8 * NP) if opening else 0)
            pacer.spread([unit[0] for unit in units], first, span_q - 11, w1)
            pacer.spread([unit[1] for unit in units], first + 10, span_q - 1, w2)
            nxt = (g + 1) % NG
            if opening:
                pacer.spread(second_pair, W_NORM, slot_q - 8, W_NORM)
                for p in range(2, NP):
                    transposes, normalize = input_jobs(p)
                    pacer.spread(transposes, (p - 2) * slot_q + W_XPOSE, (p - 1) * slot_q - 4, W_XPOSE)
                    pacer.spread(normalize, (p - 1) * slot_q + W_NORM - 8, p * slot_q - 8, W_NORM)
                pacer.spread(out_weight_jobs(0, g), W_XPOSE, slot_q, W_XPOSE)
                pacer.spread(qkv_weight_jobs(0, nxt, wa_ref), span_q - 2 * slot_q + W_XPOSE, span_q - 1, W_XPOSE)
            elif rep == 0:
                @pl.when(g + 1 < NG)
                def _():
                    wait_local_weights(g + 1)

                @pl.when(g + 2 < NG)
                def _():
                    start_local_weights(g + 2)

                @pl.when(g + 1 < NG)
                def _():
                    for piece in full_weight_copies(_blk(g + 1)):
                        piece.start()

                pacer.spread(qkv_weight_jobs(0, nxt, wa_ref) + out_weight_jobs(0, g), W_XPOSE, span_q - 1, W_XPOSE)

                def copy(r):
                    def run(start):
                        wcur_ref[0, _blk(r, 8)] = _after(wa_ref[nxt + z(), _blk(r, 8)], start)
                        return _fence(wcur_ref, z())
                    return run
                pacer.spread([copy(r) for r in range(MQ // 8)], span_q - slot_q + W_COPY, span_q - 1, W_COPY)

            for p in range(NP):
                if opening and p % 2 == 0 and p + 2 < NP:
                    wait_input(p + 2)
                    wait_input(p + 3)
                    if p == 0:
                        start_inputs(6, NP)
                        start_local_weights(1)
                    if p == NP - 4:
                        wait_local_weights(1)
                        start_local_weights(2)
                        for piece in full_weight_copies(_blk(0, 256)):
                            piece.start()
                w_ref = wcur_ref.at[0] if opening or (rep == 0 and p < NP - 1) else wa_ref.at[g]
                for u in (2 * p, 2 * p + 1):
                    for i in range(2):
                        kqv = pacer.product(w_ref, _blk(i, MQ // 2), normalized(p, opening), _blk(u % 2))
                        staged[u % (2 * NS), i] = (0, u)
                        _put(lkv_refs[u % (2 * NS)].at[0], _blk(i, 64), _blk(0), kqv[:64])
                        lq_refs[u % (2 * NS)][0, _blk(i, 64)] = kqv[64:128] * QSCALE
                        _put(lkv_refs[u % (2 * NS)].at[0], _blk(i, 64), _blk(1), kqv[128:])
            assert not pacer.jobs

        if rep == 0:
            step(0)
            wcur_ref[0, :MQ] = wa_ref[1 + z(), :MQ]
        else:
            for job in last_layernorm_jobs(xa_refs):
                job(None)
        pl.loop(1 - rep, NG)(step)

    def qkv_full(rep):
        @pl.loop(0, NG, step=GPB)
        def _(g0):
            pacer = _Pacer(zero())
            pacer.spread(last_layernorm_jobs(xb_refs), W_NORM, span_q - 2 * slot_q, W_NORM)
            for h in range(GPB):
                g = g0 + h
                if rep == 0:
                    first = h * span_q + slot_q // 2
                    pacer.spread(out_weight_jobs(1, g), first, first + 3 * slot_q, W_XPOSE)
                for u in range(2 * NP):
                    kqv = [pacer.product(wb_ref.at[g], _blk(i, MQ // 2), normalized(u // 2, u // 2 == NP - 1),
                                         _blk(u % 2)) for i in range(2)]
                    for i in range(2):
                        _put(q_ref.at[g * NQ + u // 4], _blk(i, 64), _blk(u % 4), kqv[i][64:128] * QSCALE)
                        _put(v_ref.at[g], _blk(i, 64), _blk(u), kqv[i][128:])
                    k_ref[g, _blk(u, 64), :] = _bits(jnp.concatenate([x[:64] for x in kqv], axis=0).astype(BF16).T)
            assert not pacer.jobs

    def values(item, a, c):
        return _bf16(v_ref[item // NQ, _blk(a, DH // 2), _blk(c, CK)])

    def store_head(item, a, acc, total):
        both = jnp.concatenate([acc, total], axis=0)
        for j in range(BQ // 128):
            o_ref[item % NQ * (BQ // 128) + j, item // NQ * 4 + a] = both[:, _blk(j)]

    def attend(item, first, last, jobs=()):
        tops, marks, due = {}, [], [[], []]
        top = total = acc = None
        for n in range(first, last):
            ahead, a = item + (n + SKEW) // 4, (n + SKEW) % 4
            q = _bf16(q_ref[ahead, _blk(a, DH // 2), :])
            q = jnp.concatenate([q if b == a else jnp.zeros_like(q) for b in range(4)], axis=0)
            if n >= 0:
                peak = tops[n % SKEW] if n % SKEW in tops else m_ref[n % SKEW]
            unreduced, total_before, acc_before = top, total, acc
            top = total = acc = None
            for c in range(NC):
                done = due.pop(0)
                due.append([])
                if c == 1 and unreduced is not None:
                    tops[(n - 1) % SKEW] = _all8(jnp.maximum, _after(unreduced, token(marks[0])))
                    due[-1].append(token(tops[(n - 1) % SKEW]))
                at, steps = (n - first) * NC + c, (last - first) * NC
                for job in jobs[at * len(jobs) // steps:(at + 1) * len(jobs) // steps]:
                    due[-1].append(job(token(marks[0][:, :128]) if marks else None))
                if n >= 0:
                    for t in done:
                        peak = _after(peak, t)
                    peaks = [_after(peak, token(mark)) for mark in marks[::2]] or [peak] * (CK // 32)
                    p, total = _exp_scores(lambda rows: s_refs[n % 4][c + z(), rows],
                                           [peaks[i // 2] for i in range(CK // 16)], total,
                                           None if total_before is None else token(total_before))
                s = _dot(_bf16(k_ref[ahead // NQ, _blk(c, CK // 2), :]), q)
                s_refs[a][c] = s
                link, marks = marks[-1:], []
                for i, slab in enumerate(_rows8(s)):
                    top = _after(slab, token(*link) if link else None) if top is None else jnp.maximum(top, slab)
                    if i % 2:
                        marks.append(top)
                if n >= 0:
                    o = _dot(values(item + n // 4, n % 4, c), p)
                    if acc is not None:
                        acc = acc + o
                    elif acc_before is not None:
                        acc = _after(o, _bits(acc_before) & _tile(zero(), DH // 8, BQ // 128))
                    else:
                        acc = o
            if n >= 0:
                store_head(item + n // 4, n % 4, acc, total)
        tops[(last - 1) % SKEW] = _all8(jnp.maximum, top)
        for slot, peak in tops.items():
            m_ref[slot] = peak

    def last_head_jobs(a):
        item, state = NG * NQ - 1, [None, None]

        def job(c):
            def run(start):
                p, state[0] = _exp_scores(lambda rows: s_refs[a][c + z(), rows],
                                          [_after(m_ref[a % SKEW + z()], start)] * (CK // 16), state[0], None)
                o = _dot(values(item, a, c), p)
                state[1] = o if state[1] is None else state[1] + o
                return token(*[x[:, _blk(j)] for x in (state[0], state[1][-8:]) for j in range(BQ // 128)])
            return run

        def store(start):
            store_head(item, a, _after(state[1], start), state[0])
            return start
        return [job(c) for c in range(NC)], store

    def attention():
        items = NG * NQ
        trips = (items - 1) // IPB
        lead = items - 1 - trips * IPB
        attend(0, -SKEW, 4 * lead)
        pl.loop(0, trips)(lambda i: attend(lead + i * IPB, 0, 4 * IPB))
        attend(items - 1, 0, 4 - SKEW, divide_jobs(0, 0))

    span_o = 4 * D // 16

    def project(layer, t, src_refs, emit, add_jobs):
        pacer = _Pacer(zero())
        if layer:
            pacer.spread(divide_jobs(2 * t + 1, 1), W_OPERAND, span_o - W_OPERAND, W_OPERAND)
            pacer.spread(divide_jobs(jnp.minimum(2 * t + 2, NP - 1), 0), span_o + W_OPERAND, 2 * span_o - 1, W_OPERAND)
        add_jobs(pacer)
        for pp in range(2):
            attended = op_refs[pp].at[0] if layer else lo_ref.at[2 * t + pp]
            for j in range(D // MO):
                for b in range(2):
                    y = pacer.product(wo_ref.at[layer], _blk(j, MO // 2), attended, _blk(b))
                    for c in range(MO // 128):
                        f = j * (MO // 128) + c
                        emit(pp, b, f, src_refs[pp][t, b, _blk(f)] + y[_blk(c)])
        pacer.flush()
        assert not pacer.jobs

    def project_and_normalize(layer, t, src_refs, dst_refs, add_jobs):
        def emit(pp, b, f, x):
            dst_refs[pp][t, b, _blk(f)] = x

        def add_all(pacer):
            if not isinstance(t, int):
                pacer.spread(layernorm_jobs(dst_refs[1].at[t - 1], h_refs[1], t - 1), W_NORM, span_o - 1, W_NORM)
            pacer.spread(layernorm_jobs(dst_refs[0].at[t + z()], h_refs[0], t), span_o + W_NORM, 2 * span_o - 1, W_NORM)
            add_jobs(pacer)
        project(layer, t, src_refs, emit, add_all)

    def project_and_write(layer, t, src_refs, add_jobs):
        def emit(pp, b, f, x):
            io_ref[_blk(4 * t + 2 * pp + b), _blk(f)] = x.astype(BF16).T
            if b == 1 and (f + 1) % (NG // 2) == 0:
                out_copy(2 * t + pp, _blk(f // (NG // 2), HD)).start()
        project(layer, t, src_refs, emit, add_jobs)

    def out_local(rep):
        def step(t):
            def add_jobs(pacer):
                if isinstance(t, int):
                    units = local_jobs(NG - 1, staged_at_end(0), 0)[-LAG:]
                    w1, w2 = W_LOCAL[0]
                    end = span_o + 16
                    pacer.spread([unit[0] for unit in units], w1, end - 10, w1)
                    pacer.spread([unit[1] for unit in units], w1 + 10, end, w2)
                if rep == 0:
                    pacer.spread(qkv_weight_jobs(1, 2 * t, wb_ref) + qkv_weight_jobs(1, 2 * t + 1, wb_ref),
                                 W_XPOSE, 2 * span_o - 1, W_XPOSE)
            project_and_normalize(0, t, xa_refs, xb_refs, add_jobs)
        step(0)
        pl.loop(1, NP // 2)(step)

    def out_full(rep):
        def finish_attention(pacer):
            tick = MO // 16
            heads = [last_head_jobs(a) for a in range(4 - SKEW, 4)]
            slots = 2 * span_o // tick
            for i, (chunks, store) in enumerate(heads):
                for c, job in enumerate(chunks):
                    start = (i * NC + c) * slots // (SKEW * NC) * tick
                    pacer.spread([job], start + W_VALUES, start + W_VALUES, W_VALUES)
                start = min(start + W_VALUES, 2 * span_o - 1)
                pacer.spread([store], start + tick, start + tick, tick)

        def step(t, add_jobs):
            if rep == 0:
                project_and_normalize(1, t, xb_refs, xa_refs, add_jobs)
            else:
                project_and_write(1, t, xb_refs, add_jobs)
        step(0, finish_attention)
        pl.loop(1, NP // 2)(lambda t: step(t, lambda pacer: None))

    second_pair = prologue()
    for rep in range(2):
        qkv_local(rep, second_pair)
        if rep == 0:
            for whole in full_weight_copies(slice(None)):
                whole.wait()
        out_local(rep)
        qkv_full(rep)
        attention()
        out_full(rep)
    for p in range(NP):
        out_copy(p, slice(None)).wait()


@jax.jit
def pallas_interleave_layers__sliding_local_dilated__softmax_full_mha__prompt_kernel(
    A_x: jax.Array,
    A_wqkv: jax.Array,
    A_wo: jax.Array,
    B_x: jax.Array,
    B_wqkv: jax.Array,
    B_wo: jax.Array,
):
    del B_x
    assert A_x.shape == (1, S, D)
    vmem = pltpu.VMEM
    out = pl.pallas_call(
        _kernel,
        out_shape=jax.ShapeDtypeStruct((S, D), BF16),
        in_specs=[pl.BlockSpec(memory_space=pl.ANY)] * 5,
        out_specs=pl.BlockSpec(memory_space=pl.ANY),
        scratch_shapes=[
            vmem((S, D), BF16),
            vmem((NG, 4, D, 128), BF16),
            vmem((D, 3 * D), BF16),
            vmem((D, D), BF16),
            vmem((NG, MQ + 8, D), U32),
            vmem((1, MQ + 8, D), U32),
            vmem((NG, MQ + 8, D), U32),
            vmem((2, D // 2 + 8, D), U32),
            [vmem((NP // 2, 2, D, 128), F32)] * 2,
            [vmem((NP // 2, 2, D, 128), F32)] * 2,
            [vmem((NP // 2, D // 2 + 16, 256), U32)] * 2,
            vmem((NP, D // 2 + 16, 256), U32),
            vmem((2 * NP, H, DH + 8, 128), F32),
            [vmem((1, D // 2 + 16, 256), U32)] * 2,
            [vmem((1, 128, 128), F32)] * (2 * NS),
            [vmem((1, 64, 256), U32)] * (2 * NS),
            vmem((NG * NQ, 64, BQ), U32),
            vmem((NG, S // 2, 128), U32),
            vmem((NG, 64, S), U32),
            [vmem((NC, CK, BQ), F32)] * 4,
            vmem((SKEW, 8, BQ), F32),
            vmem((8, 128), U32),
            pltpu.SMEM((1,), jnp.int32),
            pltpu.SemaphoreType.DMA((NP,)),
            pltpu.SemaphoreType.DMA((NG,)),
            pltpu.SemaphoreType.DMA((2,)),
        ],
        compiler_params=pltpu.CompilerParams(vmem_limit_bytes=112 * 1024 * 1024),
        name="interleaved_attention_layers",
    )(A_x.reshape(S, D), A_wqkv, A_wo, B_wqkv, B_wo)
    return out.reshape(1, S, D)
```
